```python
import jax
import jax.numpy as jnp

def _softmax(x, axis=-1):
    return jax.nn.softmax(x, axis=axis)
def _gelu(x):
    return jax.nn.gelu(x, approximate=True)
def _silu(x):
    return jax.nn.silu(x)
def _sigmoid(x):
    return jax.nn.sigmoid(x)
def _layernorm(x, axis=-1, eps=1e-5):
    m = jnp.mean(x, axis=axis, keepdims=True)
    v = jnp.var(x, axis=axis, keepdims=True)
    return (x - m) / jnp.sqrt(v + eps)
def _scatter_add(tgt, idx, src, axis=0):
    return tgt.at[idx].add(src)
def _segment_sum(src, seg, n):
    return jax.ops.segment_sum(src, seg, n)
class _Rng:
    def __init__(self, key):
        self._k = key
    def _next(self):
        self._k, sub = jax.random.split(self._k)
        return sub
    def normal(self, shape):
        return jax.random.normal(self._next(), shape, dtype=jnp.bfloat16)
    def randint(self, lo, hi, shape):
        return jax.random.randint(self._next(), shape, lo, hi, dtype=jnp.int32)
    def uniform(self, shape, lo=0.0, hi=1.0):
        return jax.random.uniform(self._next(), shape, jnp.bfloat16, lo, hi)
    def permutation(self, n):
        return jax.random.permutation(self._next(), n)


kernel_name = 'parallel_sum__sliding_local_dilated__glu_gated_geglu__prompt'

def setup_inputs():
    _rng = _Rng(jax.random.key(int.from_bytes(__import__("os").urandom(4), "little")))
    _w = (lambda a: (lambda t: t.astype(jnp.bfloat16) if jnp.issubdtype(t.dtype, jnp.floating) else t)(jnp.asarray(a)))
    def _A_setup():
        B, S, D = 1, 2048, 1024
        return {
            "x": _w((lambda *s: _rng.normal(s) * 0.05)(B, S, D)),
            "wqkv": _w((lambda *s: _rng.normal(s) * 0.05)(D, 3 * D)),
            "wo": _w((lambda *s: _rng.normal(s) * 0.05)(D, D)),
        }
    _A_in = _A_setup()

    def _B_setup():
        B, S, Dm, Df = 1, 2048, 1024, 3584
        return {
            "x": _w((lambda *s: _rng.normal(s) * 0.05)(B, S, Dm)),
            "w_gate": _w((lambda *s: _rng.normal(s) * 0.05)(Dm, Df) * (Dm ** -0.5)),
            "w_up": _w((lambda *s: _rng.normal(s) * 0.05)(Dm, Df) * (Dm ** -0.5)),
            "w_down": _w((lambda *s: _rng.normal(s) * 0.05)(Df, Dm) * (Df ** -0.5)),
        }
    _B_in = _B_setup()

    return {
        "A_x": _A_in["x"],
        "A_wqkv": _A_in["wqkv"],
        "A_wo": _A_in["wo"],
        "B_x": _B_in["x"],
        "B_w_gate": _B_in["w_gate"],
        "B_w_up": _B_in["w_up"],
        "B_w_down": _B_in["w_down"],
    }

def reference(A_x, A_wqkv, A_wo, B_x, B_w_gate, B_w_up, B_w_down):
    def _A_ref(x, wqkv, wo):
        B, S, D = x.shape
        H = 32; Dh = D // H
        W, dil = 8, 2
        qkv = (lambda x, *d: x.transpose(*d))((x @ wqkv).reshape(B, S, 3, H, Dh), 2, 0, 3, 1, 4)
        q, k, v = qkv[0], qkv[1], qkv[2]
        scale = Dh ** -0.5
        pos = jnp.arange(S)
        off = jnp.arange(W) * dil
        idx = pos[:, None] - off[None, :]
        mask = idx >= 0
        idx_c = jnp.where(mask, idx, 0).reshape(-1)
        kg = k[:, :, idx_c, :].reshape(B, H, S, W, Dh)
        vg = v[:, :, idx_c, :].reshape(B, H, S, W, Dh)
        logits = jnp.einsum("bhsd,bhswd->bhsw", q, kg) * scale
        logits = jnp.where(mask[None, None, :, :], logits, -1e9)
        attn = _softmax(logits, axis=-1)
        o = jnp.einsum("bhsw,bhswd->bhsd", attn, vg)
        return (lambda x, *d: x.transpose(*d))(o, 0, 2, 1, 3).reshape(B, S, D) @ wo

    def _B_ref(x, w_gate, w_up, w_down):
        g = jnp.einsum("bsd,df->bsf", x, w_gate)
        u = jnp.einsum("bsd,df->bsf", x, w_up)
        h = _gelu(g) * u
        return jnp.einsum("bsf,fd->bsd", h, w_down)

    x = A_x
    xn = _layernorm(x, axis=-1)
    return x + _A_ref(xn, A_wqkv, A_wo) + _B_ref(xn, B_w_gate, B_w_up, B_w_down)
```

```python
import functools
import jax
import jax.numpy as jnp
import jax.experimental.pallas as pl
import jax.experimental.pallas.tpu as pltpu

f32, bf16, u32, i32 = jnp.float32, jnp.bfloat16, jnp.uint32, jnp.int32

HEADS = 32
WIN, DIL = 8, 2
HALO = 16
LANES = 128


def _a_combos(a11, a12, a21, a22):
    return [a11 + a22, a21 + a22, a11, a22, a11 + a12, a21 - a11, a12 - a22]


def _b_combos(b11, b12, b21, b22):
    return [b11 + b22, b11, b12 - b22, b21 - b11, b22, b11 + b12, b21 + b22]


def _c_combos(m):
    m1, m2, m3, m4, m5, m6, m7 = m
    return (m1 + m4 - m5 + m7, m3 + m5, m2 + m4, m1 - m2 + m3 + m6)


def _pack(x):
    return pltpu.bitcast(x.astype(bf16), u32)


def _unpack(x):
    return pltpu.bitcast(x, bf16)


def _dot(a, b):
    return jnp.dot(a, b, preferred_element_type=f32)


def _geglu(g, u):
    c1 = 0.7978845608028654
    c2 = c1 * 0.044715
    t = jnp.tanh(g * (c1 + c2 * (g * g)))
    return (0.5 * g) * (1.0 + t) * u


def _lane_iota(shape):
    return jax.lax.broadcasted_iota(i32, shape, 1)


def _swap_chunk_and_lane_group(src, on=None):
    n = len(src)
    g = _lane_iota(src[0].shape) // 4
    if on is None:
        cur = [src[p] if p == 0 else pltpu.roll(src[p], 4 * p, 1) for p in range(n)]
        cur = [cur[(-i) % n] for i in range(n)]
    else:
        raise NotImplementedError
    for b in range(3):
        m = (g & (1 << b)) != 0
        cur = [jnp.where(m, cur[(c - (1 << b)) % n], cur[c]) for c in range(n)]
    return [cur[c] if c == 0 else pltpu.roll(cur[c], LANES - 4 * c, 1) for c in range(n)]


def _kernel(x_hbm, wqkv_hbm, wo_hbm, wg_hbm, wu_hbm, wd_hbm, out_hbm,
            xbuf, xc, qkv, oc, acc, rawu, rawd, wc0, wc1, dc0, dc1, obuf,
            sem_x, sem_u, sem_d, sem_o, *, S, D, F, tm, ra, tmo):
    Sh, Dh = S // 2, D // 2
    TF = D // 2
    TH = TF // 2
    NF = F // TF
    NC = Sh // tm
    NCH = D // LANES
    wcs, dcs = (wc0, wc1), (dc0, dc1)
    scale = float((D // HEADS) ** -0.5)

    def x_copy(i, half):
        r = pl.ds(half * Sh + i * tm, tm)
        return pltpu.make_async_copy(x_hbm.at[r, :], xbuf.at[r, :], sem_x.at[i, half])

    def qkv_copy(t, slot):
        return pltpu.make_async_copy(wqkv_hbm.at[:, pl.ds(t * D, D)], rawu.at[slot], sem_u.at[slot, 0])

    def wo_copy(slot):
        return pltpu.make_async_copy(wo_hbm, rawu.at[slot], sem_u.at[slot, 0])

    def up_copies(f, slot):
        cps = []
        for half in range(2):
            for k, w in enumerate((wg_hbm, wu_hbm)):
                col = pl.multiple_of(f * TF + half * TH, TH)
                cps.append(pltpu.make_async_copy(
                    w.at[:, pl.ds(col, TH)],
                    rawu.at[slot, :, pl.ds((2 * half + k) * TH, TH)],
                    sem_u.at[slot, 2 * half + k]))
        return cps

    def down_copy(f, slot):
        return pltpu.make_async_copy(wd_hbm.at[pl.ds(pl.multiple_of(f * TF, TF), TF), :], rawd.at[slot],
                                     sem_d.at[slot])

    def rows(start, n):
        return pl.ds(pl.multiple_of(start, n) if not isinstance(start, int) else start, n)

    def prows(start, n):
        return pl.ds(pl.multiple_of(start // 2, n // 2) if not isinstance(start, int) else start // 2, n // 2)

    def layernorm_unit(r):
        n = 16
        xs, ys = [], []
        for half in range(2):
            x = xbuf[rows(r + half * Sh, n), :].astype(f32)
            mu = jnp.mean(x, axis=-1, keepdims=True)
            xm = x - mu
            var = jnp.mean(xm * xm, axis=-1, keepdims=True)
            xs.append(x)
            ys.append(xm * jax.lax.rsqrt(var + 1e-5))
        for c in range(Dh // LANES):
            lo = slice(c * LANES, (c + 1) * LANES)
            hi = slice(Dh + c * LANES, Dh + (c + 1) * LANES)
            a = _a_combos(ys[0][:, lo], ys[0][:, hi], ys[1][:, lo], ys[1][:, hi])
            for k in range(7):
                xc[k, prows(r, n), lo] = _pack(a[k])
            x11, x12, x21, x22 = xs[0][:, lo], xs[0][:, hi], xs[1][:, lo], xs[1][:, hi]
            z = jnp.zeros_like(x11)
            init = [z, x21, x12, z, z, x22 - x12 + x21, x11]
            for k in range(7):
                acc[k, rows(r, n), lo] = init[k]

    def up_combos_unit(rslot, wc, r, permute):
        n = 16
        tiles = []
        for half in range(2):
            rr = rows(r + half * Dh, n)
            t = [rawu[rslot, rr, c * LANES:(c + 1) * LANES] for c in range(NCH)]
            if permute:
                t = [_unpack(v) for v in _swap_chunk_and_lane_group([pltpu.bitcast(v, u32) for v in t])]
            tiles.append(t)
        for c in range(NCH // 2):
            b = _b_combos(tiles[0][c].astype(f32), tiles[0][NCH // 2 + c].astype(f32),
                          tiles[1][c].astype(f32), tiles[1][NCH // 2 + c].astype(f32))
            for k in range(7):
                wc[k, prows(r, n), c * LANES:(c + 1) * LANES] = _pack(b[k])

    def down_combos_unit(slot, dc, r):
        n = 16
        for c in range(Dh // LANES):
            lo = slice(c * LANES, (c + 1) * LANES)
            hi = slice(Dh + c * LANES, Dh + (c + 1) * LANES)
            b = _b_combos(rawd[slot, rows(r, n), lo].astype(f32), rawd[slot, rows(r, n), hi].astype(f32),
                          rawd[slot, rows(r + TH, n), lo].astype(f32), rawd[slot, rows(r + TH, n), hi].astype(f32))
            for k in range(7):
                dc[k, prows(r, n), lo] = _pack(b[k])

    def attention_rows(r, masked):
        n = 8
        lane = _lane_iota((n, LANES))
        odd = (lane & 1) != 0
        hi = (lane & 2) != 0
        q = [qkv[0, c, pl.ds(r + HALO, n), :] for c in range(NCH)]
        if masked:
            pos = r + jax.lax.broadcasted_iota(i32, (n, LANES), 0)
        logits = []
        for w in range(WIN):
            s = None
            for c in range(NCH):
                p = q[c] * qkv[1, c, pl.ds(r + HALO - DIL * w, n), :]
                s = p if s is None else s + p
            s = s + jnp.where(odd, pltpu.roll(s, 1, 1), pltpu.roll(s, LANES - 1, 1))
            s = s + jnp.where(hi, pltpu.roll(s, 2, 1), pltpu.roll(s, LANES - 2, 1))
            s = s * scale
            if masked and w > 0:
                s = jnp.where(pos >= DIL * w, s, -1e9)
            logits.append(s)
        m = functools.reduce(jnp.maximum, logits)
        e = [jnp.exp(s - m) for s in logits]
        inv = 1.0 / functools.reduce(lambda a, b: a + b, e)
        p = [v * inv for v in e]
        o = []
        for c in range(NCH):
            s = None
            for w in range(WIN):
                t = p[w] * qkv[2, c, pl.ds(r + HALO - DIL * w, n), :]
                s = t if s is None else s + t
            o.append(s)
        return _swap_chunk_and_lane_group(o)

    def attention_unit(r):
        t0, t1 = attention_rows(r, True), attention_rows(r + 8, True)
        b0, b1 = attention_rows(r + Sh, False), attention_rows(r + Sh + 8, False)
        h = NCH // 2
        for c in range(h):
            a0 = _a_combos(t0[c], t0[h + c], b0[c], b0[h + c])
            a1 = _a_combos(t1[c], t1[h + c], b1[c], b1[h + c])
            for k in range(7):
                oc[k, pl.ds(pl.multiple_of(r // 2, 8), 8), c * LANES:(c + 1) * LANES] = _pack(
                    jnp.concatenate([a0[k], a1[k]], axis=0))

    def up_products(lhs, wc, r, n):
        return [_dot(_unpack(lhs[k, prows(r, n), :]), _unpack(wc[k])) for k in range(7)]

    qkv_copy(0, 0).start()
    for i in range(NC):
        x_copy(i, 0).start()
        x_copy(i, 1).start()
    qkv_copy(1, 1).start()

    qkv_copy(0, 0).wait()

    def _pc(i, c):
        up_combos_unit(0, wc0, i * 32, True)
        up_combos_unit(0, wc0, i * 32 + 16, True)
        return c
    jax.lax.fori_loop(0, Dh // 32, _pc, 0)

    for i in range(NC):
        x_copy(i, 0).wait()
        x_copy(i, 1).wait()

        def _ln(u, c, i=i):
            layernorm_unit(i * tm + u * 32)
            layernorm_unit(i * tm + u * 32 + 16)
            return c
        jax.lax.fori_loop(0, tm // 32, _ln, 0)

    def qkv_job(t, side):
        slot = t % 2

        def body(i, c):
            r = i * tm
            c11, c12, c21, c22 = _c_combos(up_products(xc, wcs[slot], r, tm))
            for half, (lo, hi) in enumerate(((c11, c12), (c21, c22))):
                rr = pl.ds(pl.multiple_of(HALO + half * Sh + r, 8), tm)
                for ch in range(NCH // 2):
                    qkv[t, ch, rr, :] = lo[:, ch * LANES:(ch + 1) * LANES]
                    qkv[t, NCH // 2 + ch, rr, :] = hi[:, ch * LANES:(ch + 1) * LANES]
            side(i)
            return c
        jax.lax.fori_loop(0, NC, body, 0)
        for ch in range(NCH):
            qkv[t, ch, pl.ds(0, HALO), :] = jnp.broadcast_to(qkv[t, ch, pl.ds(HALO, 1), :], (HALO, LANES))

    qkv_copy(2, 0).start()
    qkv_copy(1, 1).wait()

    def up_side(slot, i, permute):
        for u in range(Dh // NC // 16):
            up_combos_unit(slot, wcs[slot], i * (Dh // NC) + 16 * u, permute)

    def down_side(slot, i):
        for u in range(TH // NC // 16):
            down_combos_unit(slot, dcs[slot], i * (TH // NC) + 16 * u)

    qkv_job(0, lambda i: up_side(1, i, True))
    for cp in up_copies(0, 1):
        cp.start()
    down_copy(0, 1).start()
    qkv_copy(2, 0).wait()
    qkv_job(1, lambda i: up_side(0, i, True))
    for cp in up_copies(1, 0):
        cp.start()
    down_copy(1, 0).start()
    for cp in up_copies(0, 1):
        cp.wait()
    down_copy(0, 1).wait()

    def _side_v(i):
        up_side(1, i, False)
        down_side(1, i)
    qkv_job(2, _side_v)

    def ffn_step(f, c):
        slot = (f + 1) % 2
        nxt = f % 2

        @pl.when(f + 2 < NF)
        def _():
            for cp in up_copies(f + 2, slot):
                cp.start()
            down_copy(f + 2, slot).start()

        @pl.when(f + 2 == NF)
        def _():
            wo_copy(slot).start()

        @pl.when(f + 1 < NF)
        def _():
            for cp in up_copies(f + 1, nxt):
                cp.wait()
            down_copy(f + 1, nxt).wait()

        @pl.when(f + 1 == NF)
        def _():
            wo_copy(nxt).wait()

        def chunks(cur):
            def body(i, c):
                r = i * tm
                cs = _c_combos(up_products(xc, wcs[cur], r, tm))
                h = _a_combos(*[_geglu(v[:, :TH], v[:, TH:]) for v in cs])
                for k in range(7):
                    acc[k, rows(r, tm), :] += _dot(h[k].astype(bf16), _unpack(dcs[cur][k]))
                up_side(1 - cur, i, False)
                down_side(1 - cur, i)
                ar = jnp.minimum((f * NC + i) * ra, Sh - ra)
                for u in range(ra // 16):
                    attention_unit(pl.multiple_of(ar + 16 * u, 16))
                return c
            jax.lax.fori_loop(0, NC, body, 0)

        pl.when(slot == 0)(lambda: chunks(0))
        pl.when(slot == 1)(lambda: chunks(1))
        return c
    jax.lax.fori_loop(0, NF, ffn_step, 0)

    oslot = (NF + 1) % 2
    NO = Sh // tmo

    def out_copy(i, half):
        r = pl.ds(pl.multiple_of(half * Sh + i * tmo, tmo), tmo)
        return pltpu.make_async_copy(obuf.at[r, :], out_hbm.at[r, :], sem_o.at[i, half])

    def obody(i, c):
        r = i * tmo
        m = up_products(oc, wcs[oslot], r, tmo)
        c11, c12, c21, c22 = _c_combos([m[k] + acc[k, rows(r, tmo), :] for k in range(7)])
        obuf[rows(r, tmo), :Dh] = c11.astype(bf16)
        obuf[rows(r, tmo), Dh:] = c12.astype(bf16)
        obuf[rows(r + Sh, tmo), :Dh] = c21.astype(bf16)
        obuf[rows(r + Sh, tmo), Dh:] = c22.astype(bf16)
        out_copy(i, 0).start()
        out_copy(i, 1).start()
        return c
    jax.lax.fori_loop(0, NO, obody, 0)
    for i in range(NO):
        out_copy(i, 0).wait()
        out_copy(i, 1).wait()


def run(A_x, A_wqkv, A_wo, B_x, B_w_gate, B_w_up, B_w_down, tm=512, ra=80, tmo=256):
    del B_x
    B, S, D = A_x.shape
    F = B_w_gate.shape[1]
    assert B == 1
    Sh, Dh = S // 2, D // 2
    TF = D // 2
    kern = functools.partial(_kernel, S=S, D=D, F=F, tm=tm, ra=ra, tmo=tmo)
    any_spec = pl.BlockSpec(memory_space=pl.ANY)
    out = pl.pallas_call(
        kern,
        in_specs=[any_spec] * 6,
        out_specs=any_spec,
        out_shape=jax.ShapeDtypeStruct((S, D), A_x.dtype),
        scratch_shapes=[
            pltpu.VMEM((S, D), bf16),
            pltpu.VMEM((7, Sh // 2, Dh), u32),
            pltpu.VMEM((3, D // LANES, HALO + S, LANES), f32),
            pltpu.VMEM((7, Sh // 2, Dh), u32),
            pltpu.VMEM((7, Sh, Dh), f32),
            pltpu.VMEM((2, D, D), bf16),
            pltpu.VMEM((2, TF, D), bf16),
            pltpu.VMEM((7, Dh // 2, Dh), u32),
            pltpu.VMEM((7, Dh // 2, Dh), u32),
            pltpu.VMEM((7, TF // 4, Dh), u32),
            pltpu.VMEM((7, TF // 4, Dh), u32),
            pltpu.VMEM((S, D), bf16),
            pltpu.SemaphoreType.DMA((Sh // tm, 2)),
            pltpu.SemaphoreType.DMA((2, 4)),
            pltpu.SemaphoreType.DMA((2,)),
            pltpu.SemaphoreType.DMA((Sh // tmo, 2)),
        ],
        compiler_params=pltpu.CompilerParams(vmem_limit_bytes=120 * 2**20),
    )(A_x.reshape(S, D), A_wqkv, A_wo, B_w_gate, B_w_up, B_w_down)
    return out.reshape(B, S, D)


@jax.jit
def pallas_parallel_sum__sliding_local_dilated__glu_gated_geglu__prompt_kernel(
        A_x, A_wqkv, A_wo, B_x, B_w_gate, B_w_up, B_w_down):
    return run(A_x, A_wqkv, A_wo, B_x, B_w_gate, B_w_up, B_w_down)
```

```python
import contextlib
import functools
import jax
import jax.numpy as jnp
import jax.experimental.pallas as pl
import jax.experimental.pallas.tpu as pltpu

f32, bf16, u32, i32 = jnp.float32, jnp.bfloat16, jnp.uint32, jnp.int32

HEADS = 32
WIN, DIL = 8, 2
HALO = 16
LANES = 128
UNIT = 16


def _a_combos(a11, a12, a21, a22):
    return [a11 + a22, a21 + a22, a11, a22, a11 + a12, a21 - a11, a12 - a22]


def _b_combos(b11, b12, b21, b22):
    return [b11 + b22, b11, b12 - b22, b21 - b11, b22, b11 + b12, b21 + b22]


def _c_combos(m):
    m1, m2, m3, m4, m5, m6, m7 = m
    return (m1 + m4 - m5 + m7, m3 + m5, m2 + m4, m1 - m2 + m3 + m6)


def _pack(x):
    return pltpu.bitcast(x.astype(bf16), u32)


def _unpack(x):
    return pltpu.bitcast(x, bf16)


def _dot(a, b):
    return jnp.dot(a, b, preferred_element_type=f32)


def _geglu(g, u):
    c1 = 0.7978845608028654
    c2 = c1 * 0.044715
    t = jnp.tanh(g * (c1 + c2 * (g * g)))
    return (0.5 * g) * (1.0 + t) * u


def _lane_iota(shape):
    return jax.lax.broadcasted_iota(i32, shape, 1)


def _swap_chunk_and_lane_group(src):
    n = len(src)
    g = _lane_iota(src[0].shape) // 4
    cur = [src[p] if p == 0 else pltpu.roll(src[p], 4 * p, 1) for p in range(n)]
    cur = [cur[(-i) % n] for i in range(n)]
    for b in range(3):
        m = (g & (1 << b)) != 0
        cur = [jnp.where(m, cur[(c - (1 << b)) % n], cur[c]) for c in range(n)]
    return [cur[c] if c == 0 else pltpu.roll(cur[c], LANES - 4 * c, 1) for c in range(n)]


def _spread(*groups, n):
    slots = [[] for _ in range(n)]
    for g in groups:
        for j, u in enumerate(g):
            slots[j * n // len(g)].append(u)
    return slots


def _kernel(x_hbm, wqkv_hbm, wo_hbm, wg_hbm, wu_hbm, wd_hbm, out_hbm,
            xbuf, xc, qkv, oc, acc, rawu, rawd, wa, wb, da, db, obuf,
            sems, *, S, D, F, tm, ochunks, only, an, pln, pun, scopes, exp):
    Sh, Dh = S // 2, D // 2
    TF = D // 2
    TH = TF // 2
    NF = F // TF
    NC = Sh // tm
    NCH = D // LANES
    HC = NCH // 2
    W0 = 2 * NC + 2 * HC
    scale = float((D // HEADS) ** -0.5)
    sc = jax.named_scope if scopes else (lambda n: contextlib.nullcontext())

    def x_copies(i):
        return [pltpu.make_async_copy(x_hbm.at[pl.ds(h * Sh + i * tm, tm), :],
                                      xbuf.at[pl.ds(h * Sh + i * tm, tm), :], sems.at[2 * i + h]) for h in range(2)]

    def q_copies(c):
        return [pltpu.make_async_copy(wqkv_hbm.at[:, pl.ds(h * Dh + c * LANES, LANES)],
                                      rawu.at[0, :, pl.ds(h * Dh + c * LANES, LANES)], sems.at[2 * NC + 2 * c + h])
                for h in range(2)]

    def qkv_copies(t, slot):
        return [pltpu.make_async_copy(wqkv_hbm.at[:, pl.ds(t * D, D)], rawu.at[slot], sems.at[W0 + 5 * slot])]

    def wo_copies():
        return [pltpu.make_async_copy(wo_hbm, rawu.at[2], sems.at[W0 + 10])]

    def ffn_copies(f, slot):
        cps = []
        for half in range(2):
            for k, w in enumerate((wg_hbm, wu_hbm)):
                col = pl.multiple_of(f * TF + half * TH, TH)
                cps.append(pltpu.make_async_copy(
                    w.at[:, pl.ds(col, TH)],
                    rawu.at[slot, :, pl.ds((2 * half + k) * TH, TH)],
                    sems.at[W0 + 5 * slot + 2 * half + k]))
        cps.append(pltpu.make_async_copy(wd_hbm.at[pl.ds(pl.multiple_of(f * TF, TF), TF), :], rawd.at[slot],
                                         sems.at[W0 + 5 * slot + 4]))
        return cps

    ostarts = [sum(ochunks[:i]) for i in range(len(ochunks))]

    def out_copies(i):
        return [pltpu.make_async_copy(obuf.at[pl.ds(h * Sh + ostarts[i], ochunks[i]), :],
                                      out_hbm.at[pl.ds(h * Sh + ostarts[i], ochunks[i]), :], sems.at[W0 + 11 + 2 * i + h])
                for h in range(2)]

    def start(cps):
        for cp in cps:
            cp.start()

    def wait(cps):
        for cp in cps:
            cp.wait()

    def rows(start, n):
        return pl.ds(start if isinstance(start, int) else pl.multiple_of(start, 16), n)

    def prows(start, n):
        return pl.ds(start // 2 if isinstance(start, int) else pl.multiple_of(start // 2, 8), n // 2)

    def lanes(c):
        return slice(c * LANES, (c + 1) * LANES)

    def chunk_refs(bufs, i):
        return [b.at[i // 2] for b in bufs[i % 2]]

    def layernorm_unit(r, n=UNIT):
        ys = []
        for half in range(2):
            x = xbuf[rows(r + half * Sh, n), :].astype(f32)
            mu = jnp.mean(x, axis=-1, keepdims=True)
            xm = x - mu
            var = jnp.mean(xm * xm, axis=-1, keepdims=True)
            ys.append(xm * jax.lax.rsqrt(var + 1e-5))
        dst = chunk_refs(xc, r // tm)
        for c in range(HC):
            lo, hi = lanes(c), lanes(HC + c)
            a = _a_combos(ys[0][:, lo], ys[0][:, hi], ys[1][:, lo], ys[1][:, hi])
            for k in range(7):
                dst[k][prows(r % tm, n), lo] = _pack(a[k])

    def residual_unit(r):
        dst = chunk_refs(acc, r // tm)
        for c in range(HC):
            lo, hi = lanes(c), lanes(HC + c)
            x11, x12 = xbuf[rows(r, UNIT), lo].astype(f32), xbuf[rows(r, UNIT), hi].astype(f32)
            x21, x22 = xbuf[rows(r + Sh, UNIT), lo].astype(f32), xbuf[rows(r + Sh, UNIT), hi].astype(f32)
            z = jnp.zeros_like(x11)
            init = [z, x21, x12, z, z, x22 - x12 + x21, x11]
            for k in range(7):
                dst[k][rows(r % tm, UNIT), lo] = init[k]

    def up_combos_unit(r, dst, src, permute=False, cols=range(HC), n=UNIT):
        top, bot = rows(r, n), rows(r + Dh, n)
        if permute:
            tiles = [[_unpack(v) for v in _swap_chunk_and_lane_group(
                [pltpu.bitcast(rawu[src, rr, lanes(c)], u32) for c in range(NCH)])] for rr in (top, bot)]
            tile = lambda half, c: tiles[half][c]
        else:
            tile = lambda half, c: rawu[src, (top, bot)[half], lanes(c)]
        for c in cols:
            b = _b_combos(tile(0, c).astype(f32), tile(0, HC + c).astype(f32),
                          tile(1, c).astype(f32), tile(1, HC + c).astype(f32))
            for k in range(7):
                dst[k][prows(r, n), lanes(c)] = _pack(b[k])

    def down_combos_unit(r, dst, src):
        top, bot = rows(r, UNIT), rows(r + TH, UNIT)
        for c in range(HC):
            lo, hi = lanes(c), lanes(HC + c)
            b = _b_combos(rawd[src, top, lo].astype(f32), rawd[src, top, hi].astype(f32),
                          rawd[src, bot, lo].astype(f32), rawd[src, bot, hi].astype(f32))
            for k in range(7):
                dst[k][prows(r, UNIT), lo] = _pack(b[k])

    def regroup_q_unit(r):
        rr = pl.ds(HALO + r, UNIT)
        v = _swap_chunk_and_lane_group([qkv[0][c, rr, :] for c in range(NCH)])
        for c in range(NCH):
            qkv[0][c, rr, :] = v[c]

    def attention_rows(r, masked, n):
        lane = _lane_iota((n, LANES))
        odd = (lane & 1) != 0
        hi = (lane & 2) != 0
        q = [qkv[0][c, pl.ds(r + HALO, n), :] for c in range(NCH)]
        if masked:
            pos = r + jax.lax.broadcasted_iota(i32, (n, LANES), 0)

        def window(t, c):
            if "rot" in exp:
                blk = qkv[t][c, pl.ds(r, n + HALO), :]
                return [blk[HALO - DIL * w:HALO - DIL * w + n] for w in range(WIN)]
            if "share" in exp:
                blks = [qkv[t][c, pl.ds(r + HALO - 8 - DIL * w, n + 8), :] for w in range(WIN // 2)]
                return [b[8:] for b in blks] + [b[:n] for b in blks]
            return [qkv[t][c, pl.ds(r + HALO - DIL * w, n), :] for w in range(WIN)]
        logits = [None] * WIN
        for c in range(NCH):
            for w, kw in enumerate(window(1, c)):
                p = q[c] * kw
                logits[w] = p if c == 0 else logits[w] + p
        for w in range(WIN):
            s = logits[w]
            s = s + jnp.where(odd, pltpu.roll(s, 1, 1), pltpu.roll(s, LANES - 1, 1))
            s = s + jnp.where(hi, pltpu.roll(s, 2, 1), pltpu.roll(s, LANES - 2, 1))
            s = s * scale
            if masked and w > 0:
                s = jnp.where(pos >= DIL * w, s, -1e9)
            logits[w] = s
        m = functools.reduce(jnp.maximum, logits)
        e = [jnp.exp(s - m) for s in logits]
        inv = 1.0 / functools.reduce(lambda a, b: a + b, e)
        p = [v * inv for v in e]
        o = []
        for c in range(NCH):
            o.append(functools.reduce(lambda a, b: a + b, [p[w] * vw for w, vw in enumerate(window(2, c))]))
        return _swap_chunk_and_lane_group(o)

    def attention_unit(r):
        top = [attention_rows(r + j, True, an) for j in range(0, UNIT, an)]
        bot = [attention_rows(r + Sh + j, False, an) for j in range(0, UNIT, an)]
        for c in range(HC):
            a = [_a_combos(t[c], t[HC + c], b[c], b[HC + c]) for t, b in zip(top, bot)]
            for k in range(7):
                oc[k][prows(r, UNIT), lanes(c)] = _pack(jnp.concatenate([v[k] for v in a], axis=0))

    def units(fn, r0, count, **kw):
        return [functools.partial(fn, r0 + j, **kw) for j in range(0, count, kw.get("n", UNIT))]

    def products(lhs, rhs, side):
        m = []
        for k in range(7):
            for u in side[k]:
                u()
            m.append(_dot(_unpack(lhs(k)), _unpack(rhs(k))))
        return m

    def qkv_chunk(t, w, i, side, c0=0, nc=HC):
        lhs = chunk_refs(xc, i)
        c11, c12, c21, c22 = _c_combos(products(
            lambda k: lhs[k][...], lambda k: w[k][:, c0 * LANES:(c0 + nc) * LANES], side))
        for half, (lo, hi) in enumerate(((c11, c12), (c21, c22))):
            rr = pl.ds(HALO + half * Sh + i * tm, tm)
            for c in range(nc):
                qkv[t][c0 + c, rr, :] = lo[:, lanes(c)]
                qkv[t][HC + c0 + c, rr, :] = hi[:, lanes(c)]

    def fill_halo(t):
        for c in range(NCH):
            qkv[t][c, pl.ds(0, HALO), :] = jnp.broadcast_to(qkv[t][c, pl.ds(HALO, 1), :], (HALO, LANES))

    def run_all(us):
        for u in us:
            u()

    none = [[]] * 7
    start(x_copies(0))
    for c in range(HC):
        start(q_copies(c))
    for i in range(1, NC):
        start(x_copies(i))
    start(qkv_copies(1, 1))

    def q_phase():
        with sc("wait_x0"):
            wait(x_copies(0))
        with sc("ln0"):
            run_all(units(layernorm_unit, 0, tm, n=pln))
        with sc("q00"):
            wait(q_copies(0))
            run_all(units(up_combos_unit, 0, Dh, dst=wa, src=0, cols=[0], n=pun))
            qkv_chunk(0, wa, 0, none, 0, 1)
        with sc("q01"):
            wait(q_copies(1) + q_copies(2) + q_copies(3))
            run_all(units(up_combos_unit, 0, Dh, dst=wa, src=0, cols=[1], n=pun))
            qkv_chunk(0, wa, 0, _spread(units(up_combos_unit, 0, Dh, dst=wa, src=0, cols=[2, 3]), n=7), 1, 1)
        with sc("q02"):
            start(qkv_copies(2, 0))
            wait(x_copies(1))
            qkv_chunk(0, wa, 0, _spread(units(layernorm_unit, tm, tm), n=7), 2, 2)
        with sc("q1"):
            wait(x_copies(2) + x_copies(3))
            qkv_chunk(0, wa, 1, _spread(units(layernorm_unit, 2 * tm, 2 * tm), n=7))
        with sc("q23"):
            wait(qkv_copies(1, 1))
            side = _spread(units(up_combos_unit, 0, Dh, dst=wb, src=1, permute=True), n=14)
            qkv_chunk(0, wa, 2, side[:7])
            qkv_chunk(0, wa, 3, side[7:])

    def k_phase():
        start(ffn_copies(0, 1))
        start(wo_copies())
        wait(qkv_copies(2, 0))
        side = _spread(units(up_combos_unit, 0, Dh, dst=wa, src=0, permute=True), units(residual_unit, 0, Sh),
                       n=7 * NC)
        for i in range(NC):
            qkv_chunk(1, wb, i, side[7 * i:7 * i + 7])
        fill_halo(1)

    def v_phase():
        start(ffn_copies(1, 0))
        wait(ffn_copies(0, 1) + wo_copies())
        side = _spread(units(up_combos_unit, 0, Dh, dst=wb, src=1), units(down_combos_unit, 0, TH, dst=db, src=1),
                       units(regroup_q_unit, 0, S), n=7 * NC)
        for i in range(NC):
            qkv_chunk(2, wa, i, side[7 * i:7 * i + 7])
        fill_halo(2)

    if only in (None, "q", "qkv"):
        q_phase()
    if only in (None, "qkv"):
        with sc("k"):
            k_phase()
        with sc("v"):
            v_phase()

    def ffn_chunk(cur, par, i, side):
        w, d = (wa, wb)[cur], (da, db)[cur]
        cs = _c_combos(products(lambda k: xc[par][k][i], lambda k: w[k][...], side[:7]))
        h = _a_combos(*[_geglu(v[:, :TH], v[:, TH:]) for v in cs])
        for k in range(7):
            run_all(side[7 + k])
            acc[par][k][i] += _dot(h[k].astype(bf16), _unpack(d[k][...]))

    def ffn_step(f, c):
        def step(cur):
            nx = 1 - cur
            nb = NC // 2
            start(ffn_copies(jnp.minimum(f + 2, NF - 1), cur))
            wait(ffn_copies(jnp.minimum(f + 1, NF - 1), nx))
            ra = -(-Sh // (NF * nb * UNIT)) * UNIT
            src = jnp.where(f + 1 < NF, nx, 2)

            def body(i, c):
                ar = jnp.minimum((f * nb + i) * ra, Sh - ra)
                side = _spread(units(up_combos_unit, i * (Dh // nb), Dh // nb, dst=(wa, wb)[nx], src=src) +
                               units(down_combos_unit, i * (TH // nb), TH // nb, dst=(da, db)[nx], src=nx),
                               units(attention_unit, pl.multiple_of(ar, UNIT), ra), n=28)
                for par in range(2):
                    ffn_chunk(cur, par, i, side[14 * par:14 * par + 14])
                return c
            with sc(f"ffn{cur}"):
                jax.lax.fori_loop(0, nb, body, 0)

        pl.when(f % 2 == 0)(lambda: step(1))
        if only is None:
            pl.when(f % 2 == 1)(lambda: step(0))
        return c
    if only in (None, "f"):
        jax.lax.fori_loop(0, NF, ffn_step, 0)
    wait(ffn_copies(NF - 1, NF % 2))

    w = (wa, wb)[(NF + 1) % 2]
    for i, (r, n) in enumerate(zip(ostarts, ochunks)):
        with sc(f"o{i}"):
            if only in (None, "o"):
                m = products(lambda k: oc[k][prows(r, n), :], lambda k: w[k][...], none)
                prev = chunk_refs(acc, r // tm)
                c11, c12, c21, c22 = _c_combos([m[k] + prev[k][rows(r % tm, n), :] for k in range(7)])
                obuf[rows(r, n), :Dh] = c11.astype(bf16)
                obuf[rows(r, n), Dh:] = c12.astype(bf16)
                obuf[rows(r + Sh, n), :Dh] = c21.astype(bf16)
                obuf[rows(r + Sh, n), Dh:] = c22.astype(bf16)
            start(out_copies(i))
    with sc("wait_out"):
        for i in range(len(ochunks)):
            wait(out_copies(i))


def run(A_x, A_wqkv, A_wo, B_x, B_w_gate, B_w_up, B_w_down, tm=256, ochunks=(256, 256, 256, 128, 128), only=None,
        an=16, pln=64, pun=64, scopes=False, exp="", flag='XLA_TPU_EVENLY_DISTRIBUTE_CRITICAL_NODES'):
    del B_x
    B, S, D = A_x.shape
    F = B_w_gate.shape[1]
    assert B == 1
    Sh, Dh = S // 2, D // 2
    TF = D // 2
    kern = functools.partial(_kernel, S=S, D=D, F=F, tm=tm, ochunks=ochunks, only=only, an=an, pln=pln, pun=pun,
                             scopes=scopes, exp=exp)
    any_spec = pl.BlockSpec(memory_space=pl.ANY)
    out = pl.pallas_call(
        kern,
        in_specs=[any_spec] * 6,
        out_specs=any_spec,
        out_shape=jax.ShapeDtypeStruct((S, D), A_x.dtype),
        scratch_shapes=[
            pltpu.VMEM((S, D), bf16),
            [[pltpu.VMEM((Sh // tm // 2, tm // 2, Dh), u32)] * 7] * 2,
            [pltpu.VMEM((D // LANES, HALO + S, LANES), f32)] * 3,
            [pltpu.VMEM((Sh // 2, Dh), u32)] * 7,
            [[pltpu.VMEM((Sh // tm // 2, tm, Dh), f32)] * 7] * 2,
            pltpu.VMEM((3, D, D), bf16),
            pltpu.VMEM((2, TF, D), bf16),
            [pltpu.VMEM((Dh // 2, Dh), u32)] * 7,
            [pltpu.VMEM((Dh // 2, Dh), u32)] * 7,
            [pltpu.VMEM((TF // 4, Dh), u32)] * 7,
            [pltpu.VMEM((TF // 4, Dh), u32)] * 7,
            pltpu.VMEM((S, D), bf16),
            pltpu.SemaphoreType.DMA((2 * (Sh // tm) + D // LANES + 11 + 2 * len(ochunks),)),
        ],
        compiler_params=pltpu.CompilerParams(
            vmem_limit_bytes=120 * 2**20, flags=None if flag is None else {k: True for k in flag.split("+")}),
    )(A_x.reshape(S, D), A_wqkv, A_wo, B_w_gate, B_w_up, B_w_down)
    return out.reshape(B, S, D)


@jax.jit
def pallas_parallel_sum__sliding_local_dilated__glu_gated_geglu__prompt_kernel(
        A_x, A_wqkv, A_wo, B_x, B_w_gate, B_w_up, B_w_down):
    return run(A_x, A_wqkv, A_wo, B_x, B_w_gate, B_w_up, B_w_down)
```

```python
import contextlib
import functools
import jax
import jax.numpy as jnp
import jax.experimental.pallas as pl
import jax.experimental.pallas.tpu as pltpu

f32, bf16, u32, i32 = jnp.float32, jnp.bfloat16, jnp.uint32, jnp.int32

HEADS = 32
WIN, DIL = 8, 2
HALO = 16
LANES = 128
UNIT = 16


def _a_combos(a11, a12, a21, a22):
    return [a11 + a22, a21 + a22, a11, a22, a11 + a12, a21 - a11, a12 - a22]


def _b_combos(b11, b12, b21, b22):
    return [b11 + b22, b11, b12 - b22, b21 - b11, b22, b11 + b12, b21 + b22]


def _c_combos(m):
    m1, m2, m3, m4, m5, m6, m7 = m
    return (m1 + m4 - m5 + m7, m3 + m5, m2 + m4, m1 - m2 + m3 + m6)


def _pack(x):
    return pltpu.bitcast(x.astype(bf16), u32)


def _unpack(x):
    return pltpu.bitcast(x, bf16)


def _dot(a, b):
    return jnp.dot(a, b, preferred_element_type=f32)


def _geglu(g, u):
    c1 = 0.7978845608028654
    c2 = c1 * 0.044715
    t = jnp.tanh(g * (c1 + c2 * (g * g)))
    return (0.5 * g) * (1.0 + t) * u


def _lane_iota(shape):
    return jax.lax.broadcasted_iota(i32, shape, 1)


def _swap_chunk_and_lane_group(src):
    n = len(src)
    g = _lane_iota(src[0].shape) // 4
    cur = [src[p] if p == 0 else pltpu.roll(src[p], 4 * p, 1) for p in range(n)]
    cur = [cur[(-i) % n] for i in range(n)]
    for b in range(3):
        m = (g & (1 << b)) != 0
        cur = [jnp.where(m, cur[(c - (1 << b)) % n], cur[c]) for c in range(n)]
    return [cur[c] if c == 0 else pltpu.roll(cur[c], LANES - 4 * c, 1) for c in range(n)]


def _spread(*groups, n):
    slots = [[] for _ in range(n)]
    for g in groups:
        for j, u in enumerate(g):
            slots[j * n // len(g)].append(u)
    return slots


def _kernel(x_hbm, wqkv_hbm, wo_hbm, wg_hbm, wu_hbm, wd_hbm, out_hbm,
            xbuf, xc, qkv, oc, acc, rawu, rawd, wa, wb, wc, dc, obuf,
            sems, *, S, D, F, tm, ochunks, only, an, pln, pun, scopes, exp):
    Sh, Dh = S // 2, D // 2
    TF = D // 2
    TH = TF // 2
    NF = F // TF
    NC = Sh // tm
    NCH = D // LANES
    HC = NCH // 2
    W0 = 2 * NC + 2 * HC
    scale = float((D // HEADS) ** -0.5)
    sc = jax.named_scope if scopes else (lambda n: contextlib.nullcontext())

    def x_copies(i):
        return [pltpu.make_async_copy(x_hbm.at[pl.ds(h * Sh + i * tm, tm), :],
                                      xbuf.at[pl.ds(h * Sh + i * tm, tm), :], sems.at[2 * i + h]) for h in range(2)]

    def q_copies(c):
        return [pltpu.make_async_copy(wqkv_hbm.at[:, pl.ds(h * Dh + c * LANES, LANES)],
                                      rawu.at[0, :, pl.ds(h * Dh + c * LANES, LANES)], sems.at[2 * NC + 2 * c + h])
                for h in range(2)]

    def qkv_copies(t, slot):
        return [pltpu.make_async_copy(wqkv_hbm.at[:, pl.ds(t * D, D)], rawu.at[slot], sems.at[W0 + 5 * slot])]

    def wo_copies():
        return [pltpu.make_async_copy(wo_hbm, rawu.at[2], sems.at[W0 + 10])]

    def ffn_copies(f, slot):
        cps = []
        for half in range(2):
            for k, w in enumerate((wg_hbm, wu_hbm)):
                col = pl.multiple_of(f * TF + half * TH, TH)
                cps.append(pltpu.make_async_copy(
                    w.at[:, pl.ds(col, TH)],
                    rawu.at[slot, :, pl.ds((2 * half + k) * TH, TH)],
                    sems.at[W0 + 5 * slot + 2 * half + k]))
        cps.append(pltpu.make_async_copy(wd_hbm.at[pl.ds(pl.multiple_of(f * TF, TF), TF), :], rawd.at[slot],
                                         sems.at[W0 + 5 * slot + 4]))
        return cps

    ostarts = [sum(ochunks[:i]) for i in range(len(ochunks))]

    def out_copies(i):
        return [pltpu.make_async_copy(obuf.at[pl.ds(h * Sh + ostarts[i], ochunks[i]), :],
                                      out_hbm.at[pl.ds(h * Sh + ostarts[i], ochunks[i]), :], sems.at[W0 + 11 + 2 * i + h])
                for h in range(2)]

    def start(cps):
        for cp in cps:
            cp.start()

    def wait(cps):
        for cp in cps:
            cp.wait()

    def rows(start, n):
        return pl.ds(start if isinstance(start, int) else pl.multiple_of(start, 16), n)

    def prows(start, n):
        return pl.ds(start // 2 if isinstance(start, int) else pl.multiple_of(start // 2, 8), n // 2)

    def lanes(c):
        return slice(c * LANES, (c + 1) * LANES)

    def chunk_refs(bufs, i):
        return bufs[i]

    def layernorm_unit(r, n=UNIT):
        ys = []
        for half in range(2):
            x = xbuf[rows(r + half * Sh, n), :].astype(f32)
            mu = jnp.mean(x, axis=-1, keepdims=True)
            xm = x - mu
            var = jnp.mean(xm * xm, axis=-1, keepdims=True)
            ys.append(xm * jax.lax.rsqrt(var + 1e-5))
        dst = chunk_refs(xc, r // tm)
        for c in range(HC):
            lo, hi = lanes(c), lanes(HC + c)
            a = _a_combos(ys[0][:, lo], ys[0][:, hi], ys[1][:, lo], ys[1][:, hi])
            for k in range(7):
                dst[k][prows(r % tm, n), lo] = _pack(a[k])

    def residual_unit(r):
        dst = chunk_refs(acc, r // tm)
        for c in range(HC):
            lo, hi = lanes(c), lanes(HC + c)
            x11, x12 = xbuf[rows(r, UNIT), lo].astype(f32), xbuf[rows(r, UNIT), hi].astype(f32)
            x21, x22 = xbuf[rows(r + Sh, UNIT), lo].astype(f32), xbuf[rows(r + Sh, UNIT), hi].astype(f32)
            z = jnp.zeros_like(x11)
            init = [z, x21, x12, z, z, x22 - x12 + x21, x11]
            for k in range(7):
                dst[k][rows(r % tm, UNIT), lo] = init[k]

    def up_combos_unit(r, dst, src, permute=False, cols=range(HC), n=UNIT):
        top, bot = rows(r, n), rows(r + Dh, n)
        if permute:
            tiles = [[_unpack(v) for v in _swap_chunk_and_lane_group(
                [pltpu.bitcast(rawu[src, rr, lanes(c)], u32) for c in range(NCH)])] for rr in (top, bot)]
            tile = lambda half, c: tiles[half][c]
        else:
            tile = lambda half, c: rawu[src, (top, bot)[half], lanes(c)]
        for c in cols:
            b = _b_combos(tile(0, c).astype(f32), tile(0, HC + c).astype(f32),
                          tile(1, c).astype(f32), tile(1, HC + c).astype(f32))
            for k in range(7):
                dst[k][prows(r, n), lanes(c)] = _pack(b[k])

    def down_combos_unit(r, dst, src):
        top, bot = rows(r, UNIT), rows(r + TH, UNIT)
        for c in range(HC):
            lo, hi = lanes(c), lanes(HC + c)
            b = _b_combos(rawd[src, top, lo].astype(f32), rawd[src, top, hi].astype(f32),
                          rawd[src, bot, lo].astype(f32), rawd[src, bot, hi].astype(f32))
            for k in range(7):
                dst[k][prows(r, UNIT), lo] = _pack(b[k])

    def regroup_q_unit(r):
        rr = pl.ds(HALO + r, UNIT)
        v = _swap_chunk_and_lane_group([qkv[0][c, rr, :] for c in range(NCH)])
        for c in range(NCH):
            qkv[0][c, rr, :] = v[c]

    def attention_rows(r, masked, n):
        lane = _lane_iota((n, LANES))
        odd = (lane & 1) != 0
        hi = (lane & 2) != 0
        q = [qkv[0][c, pl.ds(r + HALO, n), :] for c in range(NCH)]
        if masked:
            pos = r + jax.lax.broadcasted_iota(i32, (n, LANES), 0)

        def window(t, c):
            if "rot" in exp or ("rk" in exp and t == 1) or ("rv" in exp and t == 2):
                blk = qkv[t][c, pl.ds(r, n + HALO), :]
                return [blk[HALO - DIL * w:HALO - DIL * w + n] for w in range(WIN)]
            if "share" in exp:
                blks = [qkv[t][c, pl.ds(r + HALO - 8 - DIL * w, n + 8), :] for w in range(WIN // 2)]
                return [b[8:] for b in blks] + [b[:n] for b in blks]
            return [qkv[t][c, pl.ds(r + HALO - DIL * w, n), :] for w in range(WIN)]
        logits = [None] * WIN
        for c in range(NCH):
            for w, kw in enumerate(window(1, c)):
                p = q[c] * kw
                logits[w] = p if c == 0 else logits[w] + p
        for w in range(WIN):
            s = logits[w]
            s = s + jnp.where(odd, pltpu.roll(s, 1, 1), pltpu.roll(s, LANES - 1, 1))
            s = s + jnp.where(hi, pltpu.roll(s, 2, 1), pltpu.roll(s, LANES - 2, 1))
            s = s * scale
            if masked and w > 0:
                s = jnp.where(pos >= DIL * w, s, -1e9)
            logits[w] = s
        m = functools.reduce(jnp.maximum, logits)
        e = [jnp.exp(s - m) for s in logits]
        inv = 1.0 / functools.reduce(lambda a, b: a + b, e)
        p = [v * inv for v in e]
        o = []
        for c in range(NCH):
            o.append(functools.reduce(lambda a, b: a + b, [p[w] * vw for w, vw in enumerate(window(2, c))]))
        return _swap_chunk_and_lane_group(o)

    def attention_unit(r):
        top = [attention_rows(r + j, True, an) for j in range(0, UNIT, an)]
        bot = [attention_rows(r + Sh + j, False, an) for j in range(0, UNIT, an)]
        for c in range(HC):
            a = [_a_combos(t[c], t[HC + c], b[c], b[HC + c]) for t, b in zip(top, bot)]
            for k in range(7):
                oc[k][prows(r, UNIT), lanes(c)] = _pack(jnp.concatenate([v[k] for v in a], axis=0))

    def units(fn, r0, count, **kw):
        return [functools.partial(fn, r0 + j, **kw) for j in range(0, count, kw.get("n", UNIT))]

    def products(lhs, rhs, side):
        m = []
        for k in range(7):
            for u in side[k]:
                u()
            m.append(_dot(_unpack(lhs(k)), _unpack(rhs(k))))
        return m

    def qkv_chunk(t, w, i, side, c0=0, nc=HC):
        lhs = chunk_refs(xc, i)
        c11, c12, c21, c22 = _c_combos(products(
            lambda k: lhs[k][...], lambda k: w[k][:, c0 * LANES:(c0 + nc) * LANES], side))
        for half, (lo, hi) in enumerate(((c11, c12), (c21, c22))):
            rr = pl.ds(HALO + half * Sh + i * tm, tm)
            for c in range(nc):
                qkv[t][c0 + c, rr, :] = lo[:, lanes(c)]
                qkv[t][HC + c0 + c, rr, :] = hi[:, lanes(c)]

    def fill_halo(t):
        for c in range(NCH):
            qkv[t][c, pl.ds(0, HALO), :] = jnp.broadcast_to(qkv[t][c, pl.ds(HALO, 1), :], (HALO, LANES))

    def run_all(us):
        for u in us:
            u()

    none = [[]] * 7
    start(x_copies(0))
    for c in range(HC):
        start(q_copies(c))
    for i in range(1, NC):
        start(x_copies(i))
    start(qkv_copies(1, 1))

    def q_phase():
        with sc("wait_x0"):
            wait(x_copies(0))
        with sc("ln0"):
            run_all(units(layernorm_unit, 0, tm, n=pln))
        with sc("q00"):
            wait(q_copies(0))
            run_all(units(up_combos_unit, 0, Dh, dst=wa, src=0, cols=[0], n=pun))
            qkv_chunk(0, wa, 0, none, 0, 1)
        if "fine" in exp:
            with sc("q01"):
                wait(q_copies(1))
                run_all(units(up_combos_unit, 0, Dh, dst=wa, src=0, cols=[1], n=pun))
                qkv_chunk(0, wa, 0, none, 1, 1)
            with sc("q02"):
                wait(q_copies(2) + q_copies(3))
                run_all(units(up_combos_unit, 0, Dh, dst=wa, src=0, cols=[2], n=pun))
                qkv_chunk(0, wa, 0, _spread(units(up_combos_unit, 0, Dh, dst=wa, src=0, cols=[3]), n=7), 2, 1)
            with sc("q03"):
                wait(x_copies(1))
                start(qkv_copies(2, 0))
                side = _spread(units(layernorm_unit, tm, tm), n=7)
                qkv_chunk(0, wa, 0, side, 3, 1)
        else:
            with sc("q01"):
                wait(q_copies(1) + q_copies(2) + q_copies(3))
                run_all(units(up_combos_unit, 0, Dh, dst=wa, src=0, cols=[1], n=pun))
                qkv_chunk(0, wa, 0, _spread(units(up_combos_unit, 0, Dh, dst=wa, src=0, cols=[2, 3]), n=7), 1, 1)
            with sc("q02"):
                wait(x_copies(1))
                start(qkv_copies(2, 0))
                qkv_chunk(0, wa, 0, _spread(units(layernorm_unit, tm, tm), n=7), 2, 2)
        with sc("q1"):
            wait(x_copies(2) + x_copies(3))
            qkv_chunk(0, wa, 1, _spread(units(layernorm_unit, 2 * tm, 2 * tm), n=7))
        with sc("q23"):
            wait(qkv_copies(1, 1))
            side = _spread(units(up_combos_unit, 0, Dh, dst=wb, src=1, permute=True), n=14)
            qkv_chunk(0, wa, 2, side[:7])
            qkv_chunk(0, wa, 3, side[7:])

    def k_phase():
        wait(qkv_copies(2, 0))
        start(ffn_copies(0, 1))
        start(wo_copies())
        side = _spread(units(up_combos_unit, 0, Dh, dst=wa, src=0, permute=True), units(residual_unit, 0, Sh),
                       n=7 * NC)
        for i in range(NC):
            qkv_chunk(1, wb, i, side[7 * i:7 * i + 7])
        fill_halo(1)

    def v_phase():
        wait(ffn_copies(0, 1) + wo_copies())
        start(ffn_copies(1, 0))
        side = _spread(units(up_combos_unit, 0, Dh, dst=[w.at[1] for w in wc], src=1),
                       units(down_combos_unit, 0, TH, dst=[d.at[1] for d in dc], src=1),
                       units(regroup_q_unit, 0, S), n=7 * NC)
        for i in range(NC):
            qkv_chunk(2, wa, i, side[7 * i:7 * i + 7])
        fill_halo(2)

    if only in (None, "q", "qkv"):
        q_phase()
    if only in (None, "qkv"):
        with sc("k"):
            k_phase()
        with sc("v"):
            v_phase()

    def ffn_chunk(cur, i, side):
        lhs, dst = chunk_refs(xc, i), chunk_refs(acc, i)
        cs = _c_combos(products(lambda k: lhs[k][...], lambda k: wc[k][cur], side[:7]))
        h = _a_combos(*[_geglu(v[:, :TH], v[:, TH:]) for v in cs])
        for k in range(7):
            run_all(side[7 + k])
            dst[k][...] += _dot(h[k].astype(bf16), _unpack(dc[k][cur]))

    def ffn_step(f, c):
        cur, nx = (f + 1) % 2, f % 2
        wait(ffn_copies(jnp.minimum(f + 1, NF - 1), nx))
        start(ffn_copies(jnp.minimum(f + 2, NF - 1), cur))
        ra = -(-Sh // (NF * UNIT)) * UNIT
        ar = jnp.minimum(f * ra, Sh - ra)
        src = jnp.where(f + 1 < NF, nx, 2)
        side = _spread(units(attention_unit, pl.multiple_of(ar, UNIT), ra), n=14 * NC)
        ups = units(up_combos_unit, 0, Dh, dst=[w.at[nx] for w in wc], src=src)
        dns = units(down_combos_unit, 0, TH, dst=[d.at[nx] for d in dc], src=nx)
        if "p0" in exp:
            for i, (u, d) in enumerate(zip(_spread(ups, n=NC), _spread(dns, n=NC))):
                side[14 * i] += d
                side[14 * i + 7] += u
        elif "p1" in exp:
            for i, u in enumerate(_spread(ups, n=NC)):
                side[14 * i + 7] += u
            for i, d in enumerate(_spread(dns, n=NC - 1)):
                side[14 * (i + 1)] += d
        elif "p2" in exp:
            for i, u in enumerate(_spread(ups, n=NC - 1)):
                side[14 * i + 7] += u
            for i, d in enumerate(_spread(dns, n=NC - 1)):
                side[14 * (i + 1)] += d
        elif "p3" in exp:
            for i, u in enumerate(_spread(ups, n=NC - 1)):
                side[14 * (i + 1) + 7] += u
            for i, d in enumerate(_spread(dns, n=NC - 1)):
                side[14 * (i + 1)] += d
        elif "p4" in exp:
            for i, u in enumerate(_spread(ups, n=2)):
                side[14 * (i + 2) + 7] += u
            for i, d in enumerate(_spread(dns, n=2)):
                side[14 * (i + 2)] += d
        elif "p5" in exp:
            side[49] += ups
            side[42] += dns
        elif "p6" in exp:
            for i, u in enumerate(_spread(ups, n=2)):
                side[14 * (i + 2) + 7] += u
            side[42] += dns
        elif "p7" in exp:
            for i, u in enumerate(_spread(ups, n=3)):
                side[14 * (i + 1) + 7] += u
            side[42] += dns
        for i in range(NC):
            ffn_chunk(cur, i, side[14 * i:14 * i + 14])
        return c
    if only in (None, "f"):
        jax.lax.fori_loop(0, NF, ffn_step, 0)
    wait(ffn_copies(NF - 1, NF % 2))

    w = [v.at[(NF + 1) % 2] for v in wc]
    for i, (r, n) in enumerate(zip(ostarts, ochunks)):
        with sc(f"o{i}"):
            if only in (None, "o"):
                m = products(lambda k: oc[k][prows(r, n), :], lambda k: w[k][...], none)
                prev = chunk_refs(acc, r // tm)
                c11, c12, c21, c22 = _c_combos([m[k] + prev[k][rows(r % tm, n), :] for k in range(7)])
                obuf[rows(r, n), :Dh] = c11.astype(bf16)
                obuf[rows(r, n), Dh:] = c12.astype(bf16)
                obuf[rows(r + Sh, n), :Dh] = c21.astype(bf16)
                obuf[rows(r + Sh, n), Dh:] = c22.astype(bf16)
            start(out_copies(i))
    with sc("wait_out"):
        for i in range(len(ochunks)):
            wait(out_copies(i))


def run(A_x, A_wqkv, A_wo, B_x, B_w_gate, B_w_up, B_w_down, tm=256, ochunks=(256, 256, 256, 192, 64), only=None,
        an=16, pln=64, pun=64, scopes=False, exp="p4 fine", flag='XLA_TPU_EVENLY_DISTRIBUTE_CRITICAL_NODES'):
    del B_x
    B, S, D = A_x.shape
    F = B_w_gate.shape[1]
    assert B == 1
    Sh, Dh = S // 2, D // 2
    TF = D // 2
    kern = functools.partial(_kernel, S=S, D=D, F=F, tm=tm, ochunks=ochunks, only=only, an=an, pln=pln, pun=pun,
                             scopes=scopes, exp=exp)
    any_spec = pl.BlockSpec(memory_space=pl.ANY)
    out = pl.pallas_call(
        kern,
        in_specs=[any_spec] * 6,
        out_specs=any_spec,
        out_shape=jax.ShapeDtypeStruct((S, D), A_x.dtype),
        scratch_shapes=[
            pltpu.VMEM((S, D), bf16),
            [[pltpu.VMEM((tm // 2, Dh), u32)] * 7] * (Sh // tm),
            [pltpu.VMEM((D // LANES, HALO + S, LANES), f32)] * 3,
            [pltpu.VMEM((Sh // 2, Dh), u32)] * 7,
            [[pltpu.VMEM((tm, Dh), f32)] * 7] * (Sh // tm),
            pltpu.VMEM((3, D, D), bf16),
            pltpu.VMEM((2, TF, D), bf16),
            [pltpu.VMEM((Dh // 2, Dh), u32)] * 7,
            [pltpu.VMEM((Dh // 2, Dh), u32)] * 7,
            [pltpu.VMEM((2, Dh // 2, Dh), u32)] * 7,
            [pltpu.VMEM((2, TF // 4, Dh), u32)] * 7,
            pltpu.VMEM((S, D), bf16),
            pltpu.SemaphoreType.DMA((2 * (Sh // tm) + D // LANES + 11 + 2 * len(ochunks),)),
        ],
        compiler_params=pltpu.CompilerParams(
            vmem_limit_bytes=120 * 2**20, flags=None if flag is None else {k: True for k in flag.split("+")}),
    )(A_x.reshape(S, D), A_wqkv, A_wo, B_w_gate, B_w_up, B_w_down)
    return out.reshape(B, S, D)


@jax.jit
def pallas_parallel_sum__sliding_local_dilated__glu_gated_geglu__prompt_kernel(
        A_x, A_wqkv, A_wo, B_x, B_w_gate, B_w_up, B_w_down):
    return run(A_x, A_wqkv, A_wo, B_x, B_w_gate, B_w_up, B_w_down)
```

```python
import contextlib
import functools
import jax
import jax.numpy as jnp
import jax.experimental.pallas as pl
import jax.experimental.pallas.tpu as pltpu

f32, bf16, u32, i32 = jnp.float32, jnp.bfloat16, jnp.uint32, jnp.int32

HEADS = 32
WIN, DIL = 8, 2
HALO = 16
LANES = 128
UNIT = 16


def _a_combos(a11, a12, a21, a22):
    return [a11 + a22, a21 + a22, a11, a22, a11 + a12, a21 - a11, a12 - a22]


def _b_combos(b11, b12, b21, b22):
    return [b11 + b22, b11, b12 - b22, b21 - b11, b22, b11 + b12, b21 + b22]


def _c_combos(m):
    m1, m2, m3, m4, m5, m6, m7 = m
    return (m1 + m4 - m5 + m7, m3 + m5, m2 + m4, m1 - m2 + m3 + m6)


def _pack(x):
    return pltpu.bitcast(x.astype(bf16), u32)


def _unpack(x):
    return pltpu.bitcast(x, bf16)


def _dot(a, b):
    return jnp.dot(a, b, preferred_element_type=f32)


def _geglu(g, u):
    c1 = 0.7978845608028654
    c2 = c1 * 0.044715
    t = jnp.tanh(g * (c1 + c2 * (g * g)))
    return (0.5 * g) * (1.0 + t) * u


def _lane_iota(shape):
    return jax.lax.broadcasted_iota(i32, shape, 1)


def _swap_chunk_and_lane_group(src):
    n = len(src)
    g = _lane_iota(src[0].shape) // 4
    cur = [src[p] if p == 0 else pltpu.roll(src[p], 4 * p, 1) for p in range(n)]
    cur = [cur[(-i) % n] for i in range(n)]
    for b in range(3):
        m = (g & (1 << b)) != 0
        cur = [jnp.where(m, cur[(c - (1 << b)) % n], cur[c]) for c in range(n)]
    return [cur[c] if c == 0 else pltpu.roll(cur[c], LANES - 4 * c, 1) for c in range(n)]


def _spread(*groups, n):
    slots = [[] for _ in range(n)]
    for g in groups:
        for j, u in enumerate(g):
            slots[j * n // len(g)].append(u)
    return slots


def _kernel(x_hbm, wqkv_hbm, wo_hbm, wg_hbm, wu_hbm, wd_hbm, out_hbm,
            xbuf, xc, qkv, oc, acc, rawu, rawd, wa, wb, wc, dc, obuf,
            sems, *, S, D, F, tm, ochunks, only, an, pln, pun, scopes, exp, kv, vmid, nx0, oa):
    Sh, Dh = S // 2, D // 2
    TF = D // 2
    TH = TF // 2
    NF = F // TF
    NC = Sh // tm
    NCH = D // LANES
    HC = NCH // 2
    W0 = 2 * NC + 2 * HC
    scale = float((D // HEADS) ** -0.5)
    sc = jax.named_scope if scopes else (lambda n: contextlib.nullcontext())

    def x_copies(i):
        return [pltpu.make_async_copy(x_hbm.at[pl.ds(h * Sh + i * tm, tm), :],
                                      xbuf.at[pl.ds(h * Sh + i * tm, tm), :], sems.at[2 * i + h]) for h in range(2)]

    def q_copies(c):
        return [pltpu.make_async_copy(wqkv_hbm.at[:, pl.ds(h * Dh + c * LANES, LANES)],
                                      rawu.at[0, :, pl.ds(h * Dh + c * LANES, LANES)], sems.at[2 * NC + 2 * c + h])
                for h in range(2)]

    def qkv_copies(t, slot):
        return [pltpu.make_async_copy(wqkv_hbm.at[:, pl.ds(t * D, D)], rawu.at[slot], sems.at[W0 + 5 * slot])]

    def wo_copies():
        return [pltpu.make_async_copy(wo_hbm, rawu.at[2], sems.at[W0 + 10])]

    def ffn_copies(f, slot):
        cps = []
        for half in range(2):
            for k, w in enumerate((wg_hbm, wu_hbm)):
                col = pl.multiple_of(f * TF + half * TH, TH)
                cps.append(pltpu.make_async_copy(
                    w.at[:, pl.ds(col, TH)],
                    rawu.at[slot, :, pl.ds((2 * half + k) * TH, TH)],
                    sems.at[W0 + 5 * slot + 2 * half + k]))
        cps.append(pltpu.make_async_copy(wd_hbm.at[pl.ds(pl.multiple_of(f * TF, TF), TF), :], rawd.at[slot],
                                         sems.at[W0 + 5 * slot + 4]))
        return cps

    ostarts = [sum(ochunks[:i]) for i in range(len(ochunks))]

    def out_copies(i):
        return [pltpu.make_async_copy(obuf.at[pl.ds(h * Sh + ostarts[i], ochunks[i]), :],
                                      out_hbm.at[pl.ds(h * Sh + ostarts[i], ochunks[i]), :], sems.at[W0 + 11 + 2 * i + h])
                for h in range(2)]

    def start(cps):
        for cp in cps:
            cp.start()

    def wait(cps):
        for cp in cps:
            cp.wait()

    def rows(start, n):
        return pl.ds(start if isinstance(start, int) else pl.multiple_of(start, 16), n)

    def prows(start, n):
        return pl.ds(start // 2 if isinstance(start, int) else pl.multiple_of(start // 2, 8), n // 2)

    def lanes(c):
        return slice(c * LANES, (c + 1) * LANES)

    def chunk_refs(bufs, i):
        return bufs[i]

    def layernorm_unit(r, n=UNIT):
        ys = []
        for half in range(2):
            x = xbuf[rows(r + half * Sh, n), :].astype(f32)
            mu = jnp.mean(x, axis=-1, keepdims=True)
            xm = x - mu
            var = jnp.mean(xm * xm, axis=-1, keepdims=True)
            ys.append(xm * jax.lax.rsqrt(var + 1e-5))
        dst = chunk_refs(xc, r // tm)
        for c in range(HC):
            lo, hi = lanes(c), lanes(HC + c)
            a = _a_combos(ys[0][:, lo], ys[0][:, hi], ys[1][:, lo], ys[1][:, hi])
            for k in range(7):
                dst[k][prows(r % tm, n), lo] = _pack(a[k])

    def residual_unit(r):
        dst = chunk_refs(acc, r // tm)
        for c in range(HC):
            lo, hi = lanes(c), lanes(HC + c)
            x11, x12 = xbuf[rows(r, UNIT), lo].astype(f32), xbuf[rows(r, UNIT), hi].astype(f32)
            x21, x22 = xbuf[rows(r + Sh, UNIT), lo].astype(f32), xbuf[rows(r + Sh, UNIT), hi].astype(f32)
            z = jnp.zeros_like(x11)
            init = [z, x21, x12, z, z, x22 - x12 + x21, x11]
            for k in range(7):
                dst[k][rows(r % tm, UNIT), lo] = init[k]

    def up_combos_unit(r, dst, src, permute=False, cols=range(HC), n=UNIT):
        top, bot = rows(r, n), rows(r + Dh, n)
        if permute:
            tiles = [[_unpack(v) for v in _swap_chunk_and_lane_group(
                [pltpu.bitcast(rawu[src, rr, lanes(c)], u32) for c in range(NCH)])] for rr in (top, bot)]
            tile = lambda half, c: tiles[half][c]
        else:
            tile = lambda half, c: rawu[src, (top, bot)[half], lanes(c)]
        for c in cols:
            b = _b_combos(tile(0, c).astype(f32), tile(0, HC + c).astype(f32),
                          tile(1, c).astype(f32), tile(1, HC + c).astype(f32))
            for k in range(7):
                dst[k][prows(r, n), lanes(c)] = _pack(b[k])

    def down_combos_unit(r, dst, src):
        top, bot = rows(r, UNIT), rows(r + TH, UNIT)
        for c in range(HC):
            lo, hi = lanes(c), lanes(HC + c)
            b = _b_combos(rawd[src, top, lo].astype(f32), rawd[src, top, hi].astype(f32),
                          rawd[src, bot, lo].astype(f32), rawd[src, bot, hi].astype(f32))
            for k in range(7):
                dst[k][prows(r, UNIT), lo] = _pack(b[k])

    def regroup_q_unit(r, n=UNIT):
        rr = pl.ds(HALO + r, n)
        v = _swap_chunk_and_lane_group([qkv[0][c, rr, :] for c in range(NCH)])
        for c in range(NCH):
            qkv[0][c, rr, :] = v[c]

    def attention_rows(r, masked, n):
        lane = _lane_iota((n, LANES))
        odd = (lane & 1) != 0
        hi = (lane & 2) != 0
        q = [qkv[0][c, pl.ds(r + HALO, n), :] for c in range(NCH)]
        if masked:
            pos = r + jax.lax.broadcasted_iota(i32, (n, LANES), 0)

        def window(t, c):
            if "rot" in exp or ("rk" in exp and t == 1) or ("rv" in exp and t == 2):
                blk = qkv[t][c, pl.ds(r, n + HALO), :]
                return [blk[HALO - DIL * w:HALO - DIL * w + n] for w in range(WIN)]
            if "share" in exp:
                blks = [qkv[t][c, pl.ds(r + HALO - 8 - DIL * w, n + 8), :] for w in range(WIN // 2)]
                return [b[8:] for b in blks] + [b[:n] for b in blks]
            return [qkv[t][c, pl.ds(r + HALO - DIL * w, n), :] for w in range(WIN)]
        logits = [None] * WIN
        for c in range(NCH):
            for w, kw in enumerate(window(1, c)):
                p = q[c] * kw
                logits[w] = p if c == 0 else logits[w] + p
        for w in range(WIN):
            s = logits[w]
            s = s + jnp.where(odd, pltpu.roll(s, 1, 1), pltpu.roll(s, LANES - 1, 1))
            s = s + jnp.where(hi, pltpu.roll(s, 2, 1), pltpu.roll(s, LANES - 2, 1))
            s = s * scale
            if masked and w > 0:
                s = jnp.where(pos >= DIL * w, s, -1e9)
            logits[w] = s
        m = functools.reduce(jnp.maximum, logits)
        e = [jnp.exp(s - m) for s in logits]
        inv = 1.0 / functools.reduce(lambda a, b: a + b, e)
        p = [v * inv for v in e]
        o = []
        for c in range(NCH):
            o.append(functools.reduce(lambda a, b: a + b, [p[w] * vw for w, vw in enumerate(window(2, c))]))
        return _swap_chunk_and_lane_group(o)

    def attention_unit(r):
        top = [attention_rows(r + j, True, an) for j in range(0, UNIT, an)]
        bot = [attention_rows(r + Sh + j, False, an) for j in range(0, UNIT, an)]
        for c in range(HC):
            a = [_a_combos(t[c], t[HC + c], b[c], b[HC + c]) for t, b in zip(top, bot)]
            for k in range(7):
                oc[k][prows(r, UNIT), lanes(c)] = _pack(jnp.concatenate([v[k] for v in a], axis=0))

    def units(fn, r0, count, **kw):
        return [functools.partial(fn, r0 + j, **kw) for j in range(0, count, kw.get("n", UNIT))]

    def products(lhs, rhs, side):
        m = []
        for k in range(7):
            for u in side[k]:
                u()
            m.append(_dot(_unpack(lhs(k)), _unpack(rhs(k))))
        return m

    def qkv_chunk(t, w, i, side, c0=0, nc=HC):
        lhs = chunk_refs(xc, i)
        c11, c12, c21, c22 = _c_combos(products(
            lambda k: lhs[k][...], lambda k: w[k][:, c0 * LANES:(c0 + nc) * LANES], side))
        for half, (lo, hi) in enumerate(((c11, c12), (c21, c22))):
            rr = pl.ds(HALO + half * Sh + i * tm, tm)
            for c in range(nc):
                qkv[t][c0 + c, rr, :] = lo[:, lanes(c)]
                qkv[t][HC + c0 + c, rr, :] = hi[:, lanes(c)]

    def fill_halo(t):
        for c in range(NCH):
            qkv[t][c, pl.ds(0, HALO), :] = jnp.broadcast_to(qkv[t][c, pl.ds(HALO, 1), :], (HALO, LANES))

    def run_all(us):
        for u in us:
            u()

    none = [[]] * 7
    def x0_copies(j):
        n = tm // nx0
        return [pltpu.make_async_copy(x_hbm.at[pl.ds(h * Sh + j * n, n), :], xbuf.at[pl.ds(h * Sh + j * n, n), :],
                                      sems.at[W0 + 11 + 2 * len(ochunks) + 2 * j + h]) for h in range(2)]
    for j in range(nx0):
        start(x0_copies(j))
    for c in range(HC):
        start(q_copies(c))
    for i in range(1, NC):
        start(x_copies(i))
    start(qkv_copies(1, 1))

    def q_phase():
        def wq(cols):
            return units(up_combos_unit, 0, Dh, dst=wa, src=0, cols=cols, n=pun)
        for j in range(nx0):
            with sc(f"ln0_{j}"):
                wait(x0_copies(j))
                run_all(units(layernorm_unit, j * (tm // nx0), tm // nx0, n=pln))
        if "s1" in exp:
            with sc("q00"):
                wait(q_copies(0) + q_copies(1))
                run_all(wq([0]))
                qkv_chunk(0, wa, 0, _spread(wq([1]), n=7), 0, 1)
            with sc("q01"):
                wait(q_copies(2) + q_copies(3))
                qkv_chunk(0, wa, 0, _spread(wq([2, 3]), n=7), 1, 1)
            with sc("q02"):
                wait(x_copies(1))
                start(qkv_copies(2, 0))
                qkv_chunk(0, wa, 0, _spread(units(layernorm_unit, tm, tm), n=7), 2, 2)
        elif "s2" in exp:
            with sc("q00"):
                wait(q_copies(0))
                run_all(wq([0]))
                qkv_chunk(0, wa, 0, none, 0, 1)
            with sc("q01"):
                wait(q_copies(1) + q_copies(2))
                run_all(wq([1]))
                qkv_chunk(0, wa, 0, _spread(wq([2]), n=7), 1, 1)
            with sc("q02"):
                wait(q_copies(3) + x_copies(1))
                start(qkv_copies(2, 0))
                side = _spread(units(layernorm_unit, tm, tm), n=14)
                side[0] = wq([3]) + side[0]
                qkv_chunk(0, wa, 0, side[:7], 2, 1)
                qkv_chunk(0, wa, 0, side[7:], 3, 1)
        else:
            with sc("q00"):
                wait(q_copies(0))
                run_all(wq([0]))
                qkv_chunk(0, wa, 0, none, 0, 1)
            with sc("q01"):
                wait(q_copies(1))
                run_all(wq([1]))
                qkv_chunk(0, wa, 0, none, 1, 1)
            with sc("q02"):
                wait(q_copies(2) + q_copies(3))
                run_all(wq([2]))
                qkv_chunk(0, wa, 0, _spread(wq([3]), n=7), 2, 1)
            with sc("q03"):
                wait(x_copies(1))
                start(qkv_copies(2, 0))
                side = _spread(units(layernorm_unit, tm, tm), n=7)
                qkv_chunk(0, wa, 0, side, 3, 1)
        kc = units(up_combos_unit, 0, Dh, dst=wb, src=1, permute=True)
        if "x3l" in exp:
            with sc("q1"):
                wait(x_copies(2))
                qkv_chunk(0, wa, 1, _spread(units(layernorm_unit, 2 * tm, tm), n=7))
            with sc("q23"):
                wait(x_copies(3) + qkv_copies(1, 1))
                side = _spread(kc, n=14)
                for s, g in zip(side, _spread(units(layernorm_unit, 3 * tm, tm), n=7)):
                    s += g
                qkv_chunk(0, wa, 2, side[:7])
                qkv_chunk(0, wa, 3, side[7:])
        else:
            with sc("q1"):
                wait(x_copies(2) + x_copies(3))
                qkv_chunk(0, wa, 1, _spread(units(layernorm_unit, 2 * tm, 2 * tm), n=7))
            with sc("q23"):
                wait(qkv_copies(1, 1))
                side = _spread(kc, n=14)
                qkv_chunk(0, wa, 2, side[:7])
                qkv_chunk(0, wa, 3, side[7:])

    res = units(residual_unit, 0, Sh)
    reg = units(regroup_q_unit, 0, S, **({"n": 32} if "r32" in exp else {}))
    nres, nreg = int(len(res) * kv[0]), int(len(reg) * kv[1])

    def k_phase():
        wait(qkv_copies(2, 0))
        start(ffn_copies(0, 1) + wo_copies())
        groups = [units(up_combos_unit, 0, Dh, dst=wa, src=0, permute=True), res[:nres], reg[:nreg]]
        side = _spread(*[g for g in groups if g], n=7 * NC)
        for i in range(NC):
            qkv_chunk(1, wb, i, side[7 * i:7 * i + 7])
        fill_halo(1)

    def v_phase():
        def sync():
            wait(ffn_copies(0, 1) + wo_copies())
            start(ffn_copies(1, 0))
        wts = [units(up_combos_unit, 0, Dh, dst=[w.at[1] for w in wc], src=1),
               units(down_combos_unit, 0, TH, dst=[d.at[1] for d in dc], src=1)]
        first = vmid
        side = _spread(*[g for g in (res[nres:], reg[nreg:]) if g], n=7 * NC)
        for s, g in zip(side[first:], _spread(*wts, n=7 * NC - first)):
            s += g
        side[first].insert(0, sync)
        for i in range(NC):
            qkv_chunk(2, wa, i, side[7 * i:7 * i + 7])
        fill_halo(2)

    if only in (None, "q", "qkv"):
        q_phase()
    if only in (None, "qkv", "kv"):
        if "blk" in exp:
            pl.when(pl.program_id(0) == 0)(k_phase)
            pl.when(pl.program_id(0) == 0)(v_phase)
        else:
            with sc("k"):
                k_phase()
            with sc("v"):
                v_phase()

    def ffn_chunk(cur, i, side):
        lhs, dst = chunk_refs(xc, i), chunk_refs(acc, i)
        cs = _c_combos(products(lambda k: lhs[k][...], lambda k: wc[k][cur], side[:7]))
        h = _a_combos(*[_geglu(v[:, :TH], v[:, TH:]) for v in cs])
        for k in range(7):
            run_all(side[7 + k])
            dst[k][...] += _dot(h[k].astype(bf16), _unpack(dc[k][cur]))

    ra = Sh // (NF * UNIT) * UNIT if "a9" in exp else -(-Sh // (NF * UNIT)) * UNIT

    def ffn_step(f, c):
        cur, nx = (f + 1) % 2, f % 2
        wait(ffn_copies(jnp.minimum(f + 1, NF - 1), nx))
        ar = jnp.minimum(f * ra, Sh - ra)
        src = jnp.where(f + 1 < NF, nx, 2)
        side = _spread(units(attention_unit, pl.multiple_of(ar, UNIT), ra), n=14 * NC)
        ups = units(up_combos_unit, 0, Dh, dst=[w.at[nx] for w in wc], src=src)
        dns = units(down_combos_unit, 0, TH, dst=[d.at[nx] for d in dc], src=nx)
        for i, (u, d) in enumerate(zip(_spread(ups, n=2), _spread(dns, n=2))):
            side[14 * (i + NC - 2)] += d
            side[14 * (i + NC - 2) + 7] += u
        side[2].insert(0, functools.partial(start, ffn_copies(jnp.minimum(f + 2, NF - 1), cur)))
        for i in range(NC):
            ffn_chunk(cur, i, side[14 * i:14 * i + 14])
        return c
    if only in (None, "f"):
        jax.lax.fori_loop(0, NF, ffn_step, 0)
    wait(ffn_copies(NF - 1, NF % 2))

    w = [v.at[(NF + 1) % 2] for v in wc]
    for i, (r, n) in enumerate(zip(ostarts, ochunks)):
        with sc(f"o{i}"):
            if only in (None, "o"):
                side = _spread(units(attention_unit, NF * ra, Sh - NF * ra), n=7) if i == oa and 'a9' in exp else none
                m = products(lambda k: oc[k][prows(r, n), :], lambda k: w[k][...], side)
                prev = chunk_refs(acc, r // tm)
                c11, c12, c21, c22 = _c_combos([m[k] + prev[k][rows(r % tm, n), :] for k in range(7)])
                obuf[rows(r, n), :Dh] = c11.astype(bf16)
                obuf[rows(r, n), Dh:] = c12.astype(bf16)
                obuf[rows(r + Sh, n), :Dh] = c21.astype(bf16)
                obuf[rows(r + Sh, n), Dh:] = c22.astype(bf16)
            start(out_copies(i))
    with sc("wait_out"):
        for i in range(len(ochunks)):
            wait(out_copies(i))


def run(A_x, A_wqkv, A_wo, B_x, B_w_gate, B_w_up, B_w_down, tm=256, ochunks=(256, 256, 256, 192, 64), only=None,
        an=16, pln=64, pun=64, scopes=False, exp="fine nosc x3l", kv=(0.5, 0.5), vmid=0, nx0=2, oa=0, flag='XLA_TPU_EVENLY_DISTRIBUTE_CRITICAL_NODES'):
    del B_x
    B, S, D = A_x.shape
    F = B_w_gate.shape[1]
    assert B == 1
    Sh, Dh = S // 2, D // 2
    TF = D // 2
    kern = functools.partial(_kernel, S=S, D=D, F=F, tm=tm, ochunks=ochunks, only=only, an=an, pln=pln, pun=pun,
                             scopes=scopes, exp=exp, kv=kv, vmid=vmid, nx0=nx0, oa=oa)
    any_spec = pl.BlockSpec(memory_space=pl.ANY)
    out = pl.pallas_call(
        kern,
        grid=(1,) if 'blk' in exp else (),
        in_specs=[any_spec] * 6,
        out_specs=any_spec,
        out_shape=jax.ShapeDtypeStruct((S, D), A_x.dtype),
        scratch_shapes=[
            pltpu.VMEM((S, D), bf16),
            [[pltpu.VMEM((tm // 2, Dh), u32)] * 7] * (Sh // tm),
            [pltpu.VMEM((D // LANES, HALO + S, LANES), f32)] * 3,
            [pltpu.VMEM((Sh // 2, Dh), u32)] * 7,
            [[pltpu.VMEM((tm, Dh), f32)] * 7] * (Sh // tm),
            pltpu.VMEM((3, D, D), bf16),
            pltpu.VMEM((2, TF, D), bf16),
            [pltpu.VMEM((Dh // 2, Dh), u32)] * 7,
            [pltpu.VMEM((Dh // 2, Dh), u32)] * 7,
            [pltpu.VMEM((2, Dh // 2, Dh), u32)] * 7,
            [pltpu.VMEM((2, TF // 4, Dh), u32)] * 7,
            pltpu.VMEM((S, D), bf16),
            pltpu.SemaphoreType.DMA((2 * (Sh // tm) + D // LANES + 11 + 2 * len(ochunks) + 2 * nx0,)),
        ],
        compiler_params=pltpu.CompilerParams(
            vmem_limit_bytes=120 * 2**20, disable_bounds_checks='bc' not in exp,
            disable_semaphore_checks='nosc' in exp, flags=None if flag is None else {k: True for k in flag.split("+")}),
    )(A_x.reshape(S, D), A_wqkv, A_wo, B_w_gate, B_w_up, B_w_down)
    return out.reshape(B, S, D)


@jax.jit
def pallas_parallel_sum__sliding_local_dilated__glu_gated_geglu__prompt_kernel(
        A_x, A_wqkv, A_wo, B_x, B_w_gate, B_w_up, B_w_down):
    return run(A_x, A_wqkv, A_wo, B_x, B_w_gate, B_w_up, B_w_down)
```

```python
import functools

import jax
import jax.numpy as jnp
import jax.experimental.pallas as pl
import jax.experimental.pallas.tpu as pltpu

f32, bf16, u32, i32 = jnp.float32, jnp.bfloat16, jnp.uint32, jnp.int32

HEADS = 32
WIN, DIL = 8, 2
LN_EPS = 1e-5
MASKED = -1e9
LANES = 128
HALO = 16
UNIT = 16
WIDE = 64
TM = 256
FFN_CHUNKS = 2
X0_PARTS = 2
OUT_CHUNKS = (256, 256, 256, 192, 64)


def _lhs_sums(a11, a12, a21, a22):
    return [a11 + a22, a21 + a22, a11, a22, a11 + a12, a21 - a11, a12 - a22]


def _rhs_sums(b11, b12, b21, b22):
    return [b11 + b22, b11, b12 - b22, b21 - b11, b22, b11 + b12, b21 + b22]


def _recombine(m):
    m1, m2, m3, m4, m5, m6, m7 = m
    return (m1 + m4 - m5 + m7, m3 + m5, m2 + m4, m1 - m2 + m3 + m6)


def _pack(x):
    return pltpu.bitcast(x.astype(bf16), u32)


def _unpack(x):
    return pltpu.bitcast(x, bf16)


def _dot(a, b):
    return jnp.dot(a, b, preferred_element_type=f32)


def _geglu(g, u):
    c1 = 0.7978845608028654
    c2 = c1 * 0.044715
    t = jnp.tanh(g * (c1 + c2 * (g * g)))
    return (0.5 * g) * (1.0 + t) * u


def _lane_iota(shape):
    return jax.lax.broadcasted_iota(i32, shape, 1)


def _regroup_heads(src):
    n = len(src)
    g = _lane_iota(src[0].shape) // 4
    cur = [src[p] if p == 0 else pltpu.roll(src[p], 4 * p, 1) for p in range(n)]
    cur = [cur[(-i) % n] for i in range(n)]
    for b in range(3):
        m = (g & (1 << b)) != 0
        cur = [jnp.where(m, cur[(c - (1 << b)) % n], cur[c]) for c in range(n)]
    return [cur[c] if c == 0 else pltpu.roll(cur[c], LANES - 4 * c, 1) for c in range(n)]


def _spread(*groups, n):
    slots = [[] for _ in range(n)]
    for g in groups:
        for j, u in enumerate(g):
            slots[j * n // len(g)].append(u)
    return slots


def _units(fn, r0, count, **kw):
    return [functools.partial(fn, r0 + j, **kw) for j in range(0, count, kw.get("n", UNIT))]


def _run(items):
    for u in items:
        u()


def _start(copies):
    for cp in copies:
        cp.start()


def _wait(copies):
    for cp in copies:
        cp.wait()


def _rows(start, n):
    return pl.ds(start if isinstance(start, int) else pl.multiple_of(start, UNIT), n)


def _packed_rows(start, n):
    return pl.ds(start // 2 if isinstance(start, int) else pl.multiple_of(start // 2, UNIT // 2), n // 2)


def _lanes(c):
    return slice(c * LANES, (c + 1) * LANES)


def _products(lhs, rhs, side):
    m = []
    for k in range(7):
        _run(side[k])
        m.append(_dot(_unpack(lhs(k)), _unpack(rhs(k))))
    return m


def _kernel(x_hbm, wqkv_hbm, wo_hbm, wg_hbm, wu_hbm, wd_hbm, out_hbm,
            xbuf, xc, qkv, oc, acc, rawu, rawd, wa, wb, wc, dc, obuf, sems):
    S, D = x_hbm.shape
    F = wd_hbm.shape[0]
    Sh, Dh = S // 2, D // 2
    TF = D // 2
    TH = TF // 2
    NF = F // TF
    NC = Sh // TM
    NCH = D // LANES
    HC = NCH // 2
    scale = float((D // HEADS) ** -0.5)

    sem_q = 2 * NC
    sem_w = sem_q + 2 * HC
    sem_o = sem_w + 11
    sem_x0 = sem_o + 2 * len(OUT_CHUNKS)
    out_starts = [sum(OUT_CHUNKS[:i]) for i in range(len(OUT_CHUNKS))]

    def both_halves(src, dst, r, n, sem):
        return [pltpu.make_async_copy(src.at[pl.ds(h * Sh + r, n), :], dst.at[pl.ds(h * Sh + r, n), :],
                                      sems.at[sem + h]) for h in range(2)]

    def x0_copies(j):
        return both_halves(x_hbm, xbuf, j * (TM // X0_PARTS), TM // X0_PARTS, sem_x0 + 2 * j)

    def x_copies(i):
        return both_halves(x_hbm, xbuf, i * TM, TM, 2 * i)

    def out_copies(i):
        return both_halves(obuf, out_hbm, out_starts[i], OUT_CHUNKS[i], sem_o + 2 * i)

    def wq_copies(c):
        return [pltpu.make_async_copy(wqkv_hbm.at[:, pl.ds(h * Dh + c * LANES, LANES)],
                                      rawu.at[0, :, pl.ds(h * Dh + c * LANES, LANES)],
                                      sems.at[sem_q + 2 * c + h]) for h in range(2)]

    def wkv_copies(t, slot):
        return [pltpu.make_async_copy(wqkv_hbm.at[:, pl.ds(t * D, D)], rawu.at[slot], sems.at[sem_w + 5 * slot])]

    def wo_copies():
        return [pltpu.make_async_copy(wo_hbm, rawu.at[2], sems.at[sem_w + 10])]

    def ffn_copies(f, slot):
        copies = []
        for half in range(2):
            for k, w in enumerate((wg_hbm, wu_hbm)):
                col = pl.multiple_of(f * TF + half * TH, TH)
                copies.append(pltpu.make_async_copy(
                    w.at[:, pl.ds(col, TH)], rawu.at[slot, :, pl.ds((2 * half + k) * TH, TH)],
                    sems.at[sem_w + 5 * slot + 2 * half + k]))
        copies.append(pltpu.make_async_copy(
            wd_hbm.at[pl.ds(pl.multiple_of(f * TF, TF), TF), :], rawd.at[slot], sems.at[sem_w + 5 * slot + 4]))
        return copies

    def layernorm_unit(r, n=UNIT):
        ys = []
        for half in range(2):
            x = xbuf[_rows(r + half * Sh, n), :].astype(f32)
            mu = jnp.mean(x, axis=-1, keepdims=True)
            xm = x - mu
            var = jnp.mean(xm * xm, axis=-1, keepdims=True)
            ys.append(xm * jax.lax.rsqrt(var + LN_EPS))
        for c in range(HC):
            lo, hi = _lanes(c), _lanes(HC + c)
            a = _lhs_sums(ys[0][:, lo], ys[0][:, hi], ys[1][:, lo], ys[1][:, hi])
            for k in range(7):
                xc[r // TM][k][_packed_rows(r % TM, n), lo] = _pack(a[k])

    def residual_unit(r):
        for c in range(HC):
            lo, hi = _lanes(c), _lanes(HC + c)
            x11, x12 = xbuf[_rows(r, UNIT), lo].astype(f32), xbuf[_rows(r, UNIT), hi].astype(f32)
            x21, x22 = xbuf[_rows(r + Sh, UNIT), lo].astype(f32), xbuf[_rows(r + Sh, UNIT), hi].astype(f32)
            z = jnp.zeros_like(x11)
            init = [z, x21, x12, z, z, x22 - x12 + x21, x11]
            for k in range(7):
                acc[r // TM][k][_rows(r % TM, UNIT), lo] = init[k]

    def weight_unit(r, dst, src, regroup=False, cols=range(HC), n=UNIT):
        top, bot = _rows(r, n), _rows(r + Dh, n)
        if regroup:
            tiles = [[_unpack(v) for v in _regroup_heads(
                [pltpu.bitcast(rawu[src, rr, _lanes(c)], u32) for c in range(NCH)])] for rr in (top, bot)]
            tile = lambda half, c: tiles[half][c]
        else:
            tile = lambda half, c: rawu[src, (top, bot)[half], _lanes(c)]
        for c in cols:
            b = _rhs_sums(tile(0, c).astype(f32), tile(0, HC + c).astype(f32),
                          tile(1, c).astype(f32), tile(1, HC + c).astype(f32))
            for k in range(7):
                dst[k][_packed_rows(r, n), _lanes(c)] = _pack(b[k])

    def down_weight_unit(r, dst, src):
        top, bot = _rows(r, UNIT), _rows(r + TH, UNIT)
        for c in range(HC):
            lo, hi = _lanes(c), _lanes(HC + c)
            b = _rhs_sums(rawd[src, top, lo].astype(f32), rawd[src, top, hi].astype(f32),
                          rawd[src, bot, lo].astype(f32), rawd[src, bot, hi].astype(f32))
            for k in range(7):
                dst[k][_packed_rows(r, UNIT), lo] = _pack(b[k])

    def regroup_q_unit(r):
        rr = pl.ds(HALO + r, UNIT)
        v = _regroup_heads([qkv[0][c, rr, :] for c in range(NCH)])
        for c in range(NCH):
            qkv[0][c, rr, :] = v[c]

    def attention_rows(r, masked):
        lane = _lane_iota((UNIT, LANES))
        odd = (lane & 1) != 0
        hi = (lane & 2) != 0
        q = [qkv[0][c, pl.ds(r + HALO, UNIT), :] for c in range(NCH)]
        if masked:
            pos = r + jax.lax.broadcasted_iota(i32, (UNIT, LANES), 0)

        def window(t, c):
            return [qkv[t][c, pl.ds(r + HALO - DIL * w, UNIT), :] for w in range(WIN)]

        logits = [None] * WIN
        for c in range(NCH):
            for w, kw in enumerate(window(1, c)):
                p = q[c] * kw
                logits[w] = p if c == 0 else logits[w] + p
        for w in range(WIN):
            s = logits[w]
            s = s + jnp.where(odd, pltpu.roll(s, 1, 1), pltpu.roll(s, LANES - 1, 1))
            s = s + jnp.where(hi, pltpu.roll(s, 2, 1), pltpu.roll(s, LANES - 2, 1))
            s = s * scale
            if masked and w > 0:
                s = jnp.where(pos >= DIL * w, s, MASKED)
            logits[w] = s
        m = functools.reduce(jnp.maximum, logits)
        e = [jnp.exp(s - m) for s in logits]
        inv = 1.0 / functools.reduce(lambda a, b: a + b, e)
        p = [v * inv for v in e]
        o = [functools.reduce(lambda a, b: a + b, [p[w] * vw for w, vw in enumerate(window(2, c))])
             for c in range(NCH)]
        return _regroup_heads(o)

    def attention_unit(r):
        top = attention_rows(r, True)
        bot = attention_rows(r + Sh, False)
        for c in range(HC):
            a = _lhs_sums(top[c], top[HC + c], bot[c], bot[HC + c])
            for k in range(7):
                oc[k][_packed_rows(r, UNIT), _lanes(c)] = _pack(a[k])

    def project(t, w, i, side, c0=0, nc=HC):
        c11, c12, c21, c22 = _recombine(_products(
            lambda k: xc[i][k][...], lambda k: w[k][:, c0 * LANES:(c0 + nc) * LANES], side))
        for half, (lo, hi) in enumerate(((c11, c12), (c21, c22))):
            rr = pl.ds(HALO + half * Sh + i * TM, TM)
            for c in range(nc):
                qkv[t][c0 + c, rr, :] = lo[:, _lanes(c)]
                qkv[t][HC + c0 + c, rr, :] = hi[:, _lanes(c)]

    def fill_halo(t):
        for c in range(NCH):
            qkv[t][c, pl.ds(0, HALO), :] = jnp.broadcast_to(qkv[t][c, pl.ds(HALO, 1), :], (HALO, LANES))

    nothing = [[]] * 7

    for j in range(X0_PARTS):
        _start(x0_copies(j))
    for c in range(HC):
        _start(wq_copies(c))
    for i in range(1, NC):
        _start(x_copies(i))
    _start(wkv_copies(1, 1))

    def wq_units(c):
        return _units(weight_unit, 0, Dh, dst=wa, src=0, cols=[c], n=WIDE)

    for j in range(X0_PARTS):
        _wait(x0_copies(j))
        _run(_units(layernorm_unit, j * (TM // X0_PARTS), TM // X0_PARTS, n=WIDE))
    _wait(wq_copies(0))
    _run(wq_units(0))
    project(0, wa, 0, nothing, 0, 1)
    _wait(wq_copies(1))
    _run(wq_units(1))
    project(0, wa, 0, nothing, 1, 1)
    _wait(wq_copies(2) + wq_copies(3))
    _run(wq_units(2))
    project(0, wa, 0, _spread(wq_units(3), n=7), 2, 1)
    _wait(x_copies(1))
    _start(wkv_copies(2, 0))
    project(0, wa, 0, _spread(_units(layernorm_unit, TM, TM), n=7), 3, 1)

    _wait(x_copies(2))
    project(0, wa, 1, _spread(_units(layernorm_unit, 2 * TM, TM), n=7))

    _wait(x_copies(3))
    side = (_spread(_units(layernorm_unit, 3 * TM, TM), n=4) +
            _spread(_units(weight_unit, 0, Dh, dst=wb, src=1, regroup=True), n=10))
    side[4].insert(0, functools.partial(_wait, wkv_copies(1, 1)))
    project(0, wa, 2, side[:7])
    project(0, wa, 3, side[7:])

    residual = _units(residual_unit, 0, Sh)
    regroup_q = _units(regroup_q_unit, 0, S)
    hr, hq = len(residual) // 2, len(regroup_q) // 2

    _wait(wkv_copies(2, 0))
    _start(ffn_copies(0, 1) + wo_copies())
    side = _spread(_units(weight_unit, 0, Dh, dst=wa, src=0, regroup=True), residual[:hr], regroup_q[:hq],
                   n=7 * NC)
    for i in range(NC):
        project(1, wb, i, side[7 * i:7 * i + 7])
    fill_halo(1)

    _wait(ffn_copies(0, 1) + wo_copies())
    _start(ffn_copies(1, 0))
    side = _spread(residual[hr:], regroup_q[hq:],
                   _units(weight_unit, 0, Dh, dst=[w.at[1] for w in wc], src=1),
                   _units(down_weight_unit, 0, TH, dst=[d.at[1] for d in dc], src=1), n=7 * NC)
    for i in range(NC):
        project(2, wa, i, side[7 * i:7 * i + 7])
    fill_halo(2)

    def ffn_chunk(cur, i, side):
        ids = range(i * FFN_CHUNKS, (i + 1) * FFN_CHUNKS)
        blocks = _recombine(_products(lambda k: jnp.concatenate([xc[j][k][...] for j in ids], axis=0),
                                      lambda k: wc[k][cur], side[:7]))
        h = _lhs_sums(*[_geglu(v[:, :TH], v[:, TH:]) for v in blocks])
        for k in range(7):
            _run(side[7 + k])
            y = _dot(h[k].astype(bf16), _unpack(dc[k][cur]))
            for n, j in enumerate(ids):
                acc[j][k][...] += y[n * TM:(n + 1) * TM]

    att_rows = pl.cdiv(Sh, NF * UNIT) * UNIT

    def ffn_step(f, carry):
        cur, nxt = (f + 1) % 2, f % 2
        _wait(ffn_copies(jnp.minimum(f + 1, NF - 1), nxt))
        r0 = jnp.minimum(f * att_rows, Sh - att_rows)
        src = jnp.where(f + 1 < NF, nxt, 2)
        nf = NC // FFN_CHUNKS
        side = _spread(_units(attention_unit, pl.multiple_of(r0, UNIT), att_rows), n=14 * nf)
        side[14 * nf - 14] += _units(down_weight_unit, 0, TH, dst=[d.at[nxt] for d in dc], src=nxt)
        side[14 * nf - 7] += _units(weight_unit, 0, Dh, dst=[w.at[nxt] for w in wc], src=src)
        side[2].insert(0, functools.partial(_start, ffn_copies(jnp.minimum(f + 2, NF - 1), cur)))
        for i in range(nf):
            ffn_chunk(cur, i, side[14 * i:14 * i + 14])
        return carry

    jax.lax.fori_loop(0, NF, ffn_step, 0)
    _wait(ffn_copies(NF - 1, NF % 2))

    for i, (r, n) in enumerate(zip(out_starts, OUT_CHUNKS)):
        m = _products(lambda k: oc[k][_packed_rows(r, n), :], lambda k: wc[k][(NF + 1) % 2], nothing)
        c11, c12, c21, c22 = _recombine([m[k] + acc[r // TM][k][_rows(r % TM, n), :] for k in range(7)])
        obuf[_rows(r, n), :Dh] = c11.astype(out_hbm.dtype)
        obuf[_rows(r, n), Dh:] = c12.astype(out_hbm.dtype)
        obuf[_rows(r + Sh, n), :Dh] = c21.astype(out_hbm.dtype)
        obuf[_rows(r + Sh, n), Dh:] = c22.astype(out_hbm.dtype)
        _start(out_copies(i))
    for i in range(len(OUT_CHUNKS)):
        _wait(out_copies(i))


@jax.jit
def pallas_parallel_sum__sliding_local_dilated__glu_gated_geglu__prompt_kernel(
    A_x: jax.Array,
    A_wqkv: jax.Array,
    A_wo: jax.Array,
    B_x: jax.Array,
    B_w_gate: jax.Array,
    B_w_up: jax.Array,
    B_w_down: jax.Array,
):
    del B_x
    B, S, D = A_x.shape
    F = B_w_down.shape[0]
    Sh, Dh = S // 2, D // 2
    TF = D // 2
    NC = Sh // TM
    assert B == 1 and D == 8 * LANES and D // HEADS == 32 and F % TF == 0
    assert NC == 4 and sum(OUT_CHUNKS) == Sh
    num_sems = 2 * NC + D // LANES + 11 + 2 * len(OUT_CHUNKS) + 2 * X0_PARTS

    hbm = pl.BlockSpec(memory_space=pl.ANY)
    out = pl.pallas_call(
        _kernel,
        in_specs=[hbm] * 6,
        out_specs=hbm,
        out_shape=jax.ShapeDtypeStruct((S, D), A_x.dtype),
        scratch_shapes=[
            pltpu.VMEM((S, D), bf16),
            [[pltpu.VMEM((TM // 2, Dh), u32)] * 7] * NC,
            [pltpu.VMEM((D // LANES, HALO + S, LANES), f32)] * 3,
            [pltpu.VMEM((Sh // 2, Dh), u32)] * 7,
            [[pltpu.VMEM((TM, Dh), f32)] * 7] * NC,
            pltpu.VMEM((3, D, D), bf16),
            pltpu.VMEM((2, TF, D), bf16),
            [pltpu.VMEM((Dh // 2, Dh), u32)] * 7,
            [pltpu.VMEM((Dh // 2, Dh), u32)] * 7,
            [pltpu.VMEM((2, Dh // 2, Dh), u32)] * 7,
            [pltpu.VMEM((2, TF // 4, Dh), u32)] * 7,
            pltpu.VMEM((S, D), A_x.dtype),
            pltpu.SemaphoreType.DMA((num_sems,)),
        ],
        compiler_params=pltpu.CompilerParams(
            vmem_limit_bytes=120 * 2**20,
            disable_bounds_checks=True,
            flags={"XLA_TPU_EVENLY_DISTRIBUTE_CRITICAL_NODES": True},
        ),
    )(A_x.reshape(S, D), A_wqkv, A_wo, B_w_gate, B_w_up, B_w_down)
    return out.reshape(B, S, D)
```
